```python
import jax
import jax.numpy as jnp

def _softmax(x, axis=-1):
    return jax.nn.softmax(x, axis=axis)

def _gelu(x):
    return jax.nn.gelu(x, approximate=True)

def _silu(x):
    return jax.nn.silu(x)

def _sigmoid(x):
    return jax.nn.sigmoid(x)

def _layernorm(x, axis=-1, eps=1e-05):
    m = jnp.mean(x, axis=axis, keepdims=True)
    v = jnp.var(x, axis=axis, keepdims=True)
    return (x - m) / jnp.sqrt(v + eps)

def _scatter_add(tgt, idx, src, axis=0):
    return tgt.at[idx].add(src)

def _segment_sum(src, seg, n):
    return jax.ops.segment_sum(src, seg, n)

class _Rng:

    def __init__(self, key):
        self._k = key

    def _next(self):
        self._k, sub = jax.random.split(self._k)
        return sub

    def normal(self, shape):
        return jax.random.normal(self._next(), shape, dtype=jnp.bfloat16)

    def randint(self, lo, hi, shape):
        return jax.random.randint(self._next(), shape, lo, hi, dtype=jnp.int32)

    def uniform(self, shape, lo=0.0, hi=1.0):
        return jax.random.uniform(self._next(), shape, jnp.bfloat16, lo, hi)

    def permutation(self, n):
        return jax.random.permutation(self._next(), n)
kernel_name = 'interleave_layers__memory_aug_recurrent_mem_tr__moe_arch_mod__prompt'

def setup_inputs():
    _rng = _Rng(jax.random.key(int.from_bytes(__import__("os").urandom(4), "little")))
    _w = lambda a: (lambda t: t.astype(jnp.bfloat16) if jnp.issubdtype(t.dtype, jnp.floating) else t)(jnp.asarray(a))

    def _A_setup():
        B, S, Dm = (1, 2048, 512)
        H, Dh = (32, 128)
        M, seg = (8, 32)
        seg = min(seg, S)
        S = S // seg * seg
        return {'x': _w((lambda *s: _rng.normal(s) * 0.05)(B, S, Dm)), 'mem0': _w((lambda *s: _rng.normal(s) * 0.05)(B, M, Dm)), 'Wq': _w((lambda *s: _rng.normal(s) * 0.05)(Dm, H, Dh) * Dm ** (-0.5)), 'Wk': _w((lambda *s: _rng.normal(s) * 0.05)(Dm, H, Dh) * Dm ** (-0.5)), 'Wv': _w((lambda *s: _rng.normal(s) * 0.05)(Dm, H, Dh) * Dm ** (-0.5)), 'Wo': _w((lambda *s: _rng.normal(s) * 0.05)(H, Dh, Dm) * (H * Dh) ** (-0.5)), 'seg_len': seg}
    _A_in = _A_setup()

    def _B_setup():
        B, S, D, F, C = (1, 2048, 512, 1792, 1)
        return {'x': _w((lambda *s: _rng.normal(s) * 0.05)(B, S, D)), 'w_r': _w((lambda *s: _rng.normal(s) * 0.05)(D)), 'w_gate': _w((lambda *s: _rng.normal(s) * 0.05)(D, F)), 'w_up': _w((lambda *s: _rng.normal(s) * 0.05)(D, F)), 'w_down': _w((lambda *s: _rng.normal(s) * 0.05)(F, D))}
    _B_in = _B_setup()
    return {'A_x': _A_in['x'], 'A_mem0': _A_in['mem0'], 'A_Wq': _A_in['Wq'], 'A_Wk': _A_in['Wk'], 'A_Wv': _A_in['Wv'], 'A_Wo': _A_in['Wo'], 'A_seg_len': _A_in['seg_len'], 'B_x': _B_in['x'], 'B_w_r': _B_in['w_r'], 'B_w_gate': _B_in['w_gate'], 'B_w_up': _B_in['w_up'], 'B_w_down': _B_in['w_down']}

def reference(A_x, A_mem0, A_Wq, A_Wk, A_Wv, A_Wo, A_seg_len, B_x, B_w_r, B_w_gate, B_w_up, B_w_down):

    def _A_ref(x, mem0, Wq, Wk, Wv, Wo, seg_len):
        B, S, Dm = x.shape
        H, Dh = (Wq.shape[1], Wq.shape[2])
        M = mem0.shape[1]
        scale = Dh ** (-0.5)
        n_seg = S // seg_len
        L = M + seg_len
        idx = jnp.arange(L)
        mask = (idx[:, None] < M) | (idx[:, None] >= idx[None, :])
        mem = mem0
        outs = []
        for s in range(n_seg):
            xs = x[:, s * seg_len:(s + 1) * seg_len, :].copy()
            h = jnp.concatenate([mem, xs], axis=1)
            q = jnp.einsum('btd,dhe->bhte', h, Wq)
            k = jnp.einsum('btd,dhe->bhte', h, Wk)
            v = jnp.einsum('btd,dhe->bhte', h, Wv)
            scores = jnp.einsum('bhqe,bhke->bhqk', q, k) * scale
            scores = jnp.where(mask[None, None], scores, -1000000000.0)
            p = _softmax(scores, axis=-1)
            o = jnp.einsum('bhqk,bhke->bhqe', p, v)
            o = jnp.einsum('bhte,hed->btd', o, Wo)
            mem = o[:, :M, :].copy()
            outs.append(o[:, M:, :])
        return jnp.concatenate(outs, axis=1)

    def _B_ref(x, w_r, w_gate, w_up, w_down):
        B, S, D = x.shape
        C = 1
        r = x @ w_r
        idx = jnp.argsort(-r, axis=-1)[:, :C]
        idx_e = jnp.repeat(idx.reshape(B, C, 1), D, axis=2)
        x_sel = jnp.take_along_axis(x, idx_e, axis=1)
        g = _silu(x_sel @ w_gate)
        u = x_sel @ w_up
        y = g * u @ w_down
        r_sel = _sigmoid(jnp.take_along_axis(r, idx, axis=1))
        y = y * r_sel.reshape(B, C, 1)
        b_off = (jnp.arange(B) * S).reshape(B, 1)
        flat_idx = (idx + b_off).reshape(B * C)
        zero = (x * 0.0).reshape(B * S, D)
        upd = _scatter_add(zero, flat_idx, y.reshape(B * C, D), axis=0)
        return x + upd.reshape(B, S, D)
    x = A_x
    x = x + _A_ref(_layernorm(x, axis=-1), A_mem0, A_Wq, A_Wk, A_Wv, A_Wo, A_seg_len)
    x = x + _B_ref(_layernorm(x, axis=-1), B_w_r, B_w_gate, B_w_up, B_w_down)
    x = x + _A_ref(_layernorm(x, axis=-1), A_mem0, A_Wq, A_Wk, A_Wv, A_Wo, A_seg_len)
    x = x + _B_ref(_layernorm(x, axis=-1), B_w_r, B_w_gate, B_w_up, B_w_down)
    return x
```

```python
import functools
import numpy as np
import jax
import jax.numpy as jnp
from jax import lax
import jax.experimental.pallas as pl
import jax.experimental.pallas.tpu as pltpu

F32 = jnp.float32
BF16 = jnp.bfloat16
SEG = 32
EPS = 1e-05


LAG_S = 2
LAG_PV = 4
LAG_WO = 8


def _rb(x):
    return x.astype(BF16).astype(F32)


def _ln(x):
    d = x.shape[-1]
    mu = jnp.sum(x, axis=-1, keepdims=True) * (1.0 / d)
    c = x - mu
    var = jnp.sum(c * c, axis=-1, keepdims=True) * (1.0 / d)
    m = _rb(mu)
    v = _rb(var)
    den = _rb(jnp.sqrt(_rb(v + EPS)))
    return _rb(_rb(x - m) / den)


def _dot(a, b):
    return lax.dot_general(a, b, (((1,), (0,)), ((), ())), preferred_element_type=F32)


def _dot_nt(a, b):
    return lax.dot_general(a, b, (((1,), (1,)), ((), ())), preferred_element_type=F32)


def _kernel(x_ref, mem0_ref, wq_ref, wk_ref, wv_ref, wo_ref, wr_ref, wg_ref, wu_ref, wd_ref,
            out_ref, xa_scr, xn_scr, xb_scr, ot_scr, hn_scr, *, S, D, H, DH, M):
    L = M + SEG
    nseg = S // SEG
    scale = float(np.asarray(DH ** -0.5).astype(BF16))
    row = lax.broadcasted_iota(jnp.int32, (L, L), 0)
    col = lax.broadcasted_iota(jnp.int32, (L, L), 1)
    mask = (row < M) | (row >= col)
    wr = wr_ref[...].astype(F32)

    def hs(hd):
        return slice(hd * DH, (hd + 1) * DH)

    def layer(load_x, store_x):
        def finish(sp, best_v, best_s, valid):
            r0 = pl.multiple_of(sp * SEG, SEG)
            x1 = _rb(load_x(r0) + ot_scr[...])
            xn1 = _ln(x1)
            r = _rb(jnp.sum(xn1 * wr, axis=-1, keepdims=True))
            upd = r > best_v
            if valid is not None:
                upd = jnp.logical_and(upd, valid)
            best_v = jnp.where(upd, r, best_v)
            best_s = jnp.where(upd, sp, best_s)
            xa_scr[pl.ds(r0, SEG), :] = x1
            xn_scr[pl.ds(r0, SEG), :] = xn1
            store_x(r0, _rb(x1 + xn1))
            return best_v, best_s

        def step(s, carry):
            mem, best_v, best_s = carry
            h = jnp.concatenate([mem, hn_scr[...]], axis=0)
            q = [None] * H
            k = [None] * H
            v = [None] * H
            p = [None] * H
            il = [None] * H
            o = [None] * H
            acc = None

            def scores(hd):
                sc = _dot_nt(q[hd], k[hd]) * scale
                sc = jnp.where(mask, sc, -1e9)
                mx = jnp.max(sc, axis=-1, keepdims=True)
                e = jnp.exp(sc - mx)
                l = jnp.sum(e, axis=-1, keepdims=True)
                p[hd], il[hd] = e, pl.reciprocal(l, approx=True)

            sp = jnp.maximum(s - 1, 0)
            best_v, best_s = finish(sp, best_v, best_s, s > 0)
            sn = jnp.minimum(s + 1, nseg - 1)
            hn_next = _ln(load_x(pl.multiple_of(sn * SEG, SEG)))

            for t in range(H):
                q[t] = _dot(h, wq_ref[t])
                k[t] = _dot(h, wk_ref[t])
                if t - LAG_S >= 0:
                    scores(t - LAG_S)
            for t in range(H + LAG_WO):
                if t < H:
                    v[t] = _dot(h, wv_ref[t])
                if t < LAG_S:
                    scores(H - LAG_S + t)
                if 0 <= t - LAG_PV < H:
                    hd = t - LAG_PV
                    o[hd] = _dot(p[hd], v[hd]) * il[hd]
                if t - LAG_WO >= 0:
                    hd = t - LAG_WO
                    d = [_dot(o[hd], wo_ref[c, hs(hd), :]) for c in range(4)]
                    acc = d if acc is None else [a + b for a, b in zip(acc, d)]
            hn_scr[...] = hn_next
            res = _rb(jnp.concatenate(acc, axis=1))
            ot_scr[...] = res[M:]
            return res[:M], best_v, best_s

        hn_scr[...] = _ln(load_x(0))
        ot_scr[...] = jnp.zeros_like(ot_scr)
        init = (mem0_ref[...].astype(F32),
                jnp.full((SEG, 1), -jnp.inf, F32),
                jnp.zeros((SEG, 1), jnp.int32))
        _, best_v, best_s = lax.fori_loop(0, nseg, step, init)
        best_v, best_s = finish(nseg - 1, best_v, best_s, None)

        vmax = jnp.max(best_v, axis=0, keepdims=True)
        tok = best_s * SEG + lax.broadcasted_iota(jnp.int32, (SEG, 1), 0)
        idx = jnp.min(jnp.where(best_v == vmax, tok, S))
        idx = jnp.clip(idx, 0, S - 1)
        xs = xn_scr[pl.ds(idx, 1), :]
        x1 = xa_scr[pl.ds(idx, 1), :]
        xs8 = jnp.broadcast_to(xs, (8, D))
        g = _rb(_dot(xs8, wg_ref[...]))
        g = _rb(g * _rb(jax.nn.sigmoid(g)))
        u = _rb(_dot(xs8, wu_ref[...]))
        y = _rb(_dot(_rb(g * u), wd_ref[...]))
        y = _rb(y * _rb(jax.nn.sigmoid(vmax)))
        new = _rb(x1 + _rb(xs + y[0:1]))
        return idx, new

    def load0(r0):
        return x_ref[pl.ds(r0, SEG), :].astype(F32)

    def store0(r0, val):
        xb_scr[pl.ds(r0, SEG), :] = val

    idx, new = layer(load0, store0)
    xb_scr[pl.ds(idx, 1), :] = new

    def load1(r0):
        return xb_scr[pl.ds(r0, SEG), :]

    def store1(r0, val):
        out_ref[pl.ds(r0, SEG), :] = val.astype(BF16)

    idx, new = layer(load1, store1)
    b0 = pl.multiple_of((idx // 16) * 16, 16)
    blk = out_ref[pl.ds(b0, 16), :].astype(F32)
    rid = b0 + lax.broadcasted_iota(jnp.int32, (16, D), 0)
    out_ref[pl.ds(b0, 16), :] = jnp.where(rid == idx, new, blk).astype(BF16)


@jax.jit
def pallas_interleave_layers__memory_aug_recurrent_mem_tr__moe_arch_mod__prompt_kernel(
    A_x, A_mem0, A_Wq, A_Wk, A_Wv, A_Wo, A_seg_len, B_x, B_w_r, B_w_gate, B_w_up, B_w_down,
):
    B, S, D = A_x.shape
    _, H, DH = A_Wq.shape
    M = A_mem0.shape[1]
    assert B == 1
    kern = functools.partial(_kernel, S=S, D=D, H=H, DH=DH, M=M)
    out = pl.pallas_call(
        kern,
        out_shape=jax.ShapeDtypeStruct((S, D), BF16),
        scratch_shapes=[pltpu.VMEM((S, D), F32)] * 3
        + [pltpu.VMEM((SEG, D), F32), pltpu.VMEM((SEG, D), F32)],
        compiler_params=pltpu.CompilerParams(vmem_limit_bytes=100 * 1024 * 1024),
    )(A_x.reshape(S, D), A_mem0.reshape(M, D),
      A_Wq.transpose(1, 0, 2), A_Wk.transpose(1, 0, 2), A_Wv.transpose(1, 0, 2),
      A_Wo.reshape(H * DH, 4, D // 4).transpose(1, 0, 2), B_w_r.reshape(1, D), B_w_gate, B_w_up, B_w_down)
    return out.reshape(B, S, D)
```

```python
import functools
import numpy as np
import jax
import jax.numpy as jnp
from jax import lax
import jax.experimental.pallas as pl
import jax.experimental.pallas.tpu as pltpu

F32 = jnp.float32
BF16 = jnp.bfloat16
U32 = jnp.uint32
SEG = 32
EPS = 1e-05
G = 4
PR = 8


def _env(name, default):
    return default


U = _env("U", 4)
NFILL = _env("NFILL", 5)
PIN_LAG = _env("PIN_LAG", 4)
PIN_GAP = _env("PIN_GAP", 2)
PIN_AT = [int(t) for t in "4,8,12,16,20,24,27,29".split(",")]
SCOPES = _env("SCOPES", 0)


class _NoScope:
    def __enter__(self):
        return self

    def __exit__(self, *a):
        return False


def _scope(name):
    return jax.named_scope(name) if SCOPES else _NoScope()


def _rb(x):
    return x.astype(BF16).astype(F32)


def _ln(x):
    d = x.shape[-1]
    mu = jnp.sum(x, axis=-1, keepdims=True) * (1.0 / d)
    c = x - mu
    var = jnp.sum(c * c, axis=-1, keepdims=True) * (1.0 / d)
    m = _rb(mu)
    v = _rb(var)
    den = _rb(jnp.sqrt(_rb(v + EPS)))
    return _rb(_rb(x - m) / den)


def _w(x):
    return pltpu.bitcast(x, BF16)


def _dot(a, b):
    return lax.dot_general(a, b, (((1,), (0,)), ((), ())), preferred_element_type=F32)


def _dot_nt(a, b):
    return lax.dot_general(a, b, (((1,), (1,)), ((), ())), preferred_element_type=F32)


def _mult(r, m):
    return r if isinstance(r, int) else pl.multiple_of(r, m)


def _step_order(H, dur_qk, dur_v, lead, hold, fin_at, l_mm, l_sm):
    NG = H // G
    out = []
    t = 0
    nqk = nv = nwo = ns = npv = 0
    qk_end = [0] * H
    v_end = [0] * H
    s_end = [0] * NG
    pv_end = [0] * NG
    last = None
    fin_done = False
    while nwo < H:
        if not fin_done and t >= fin_at:
            out.append(("finish", 0))
            fin_done = True
        s_ok = ns < NG and nqk >= (ns + 1) * G and t >= qk_end[(ns + 1) * G - 1] + l_mm
        pv_ok = (npv < ns and nv >= (npv + 1) * G and t >= v_end[(npv + 1) * G - 1] + l_mm
                 and t >= s_end[npv] + l_sm)
        qk_ok = nqk < H
        v_ok = nv < H and fin_done and (nqk >= H or nv + lead < nqk)
        wo_ok = (nwo < npv * G and t >= pv_end[nwo // G] + l_mm and (nv >= H or nwo + hold < nv))
        if s_ok:
            out.append(("s", ns)); t += 40; s_end[ns] = t; ns += 1
        elif pv_ok:
            out.append(("pv", npv)); t += 40; pv_end[npv] = t; npv += 1
        else:
            cand = [c for c, ok in (("qk", qk_ok), ("v", v_ok), ("wo", wo_ok)) if ok]
            if not cand:
                t += 4
                continue
            rot = {"qk": ("v", "wo", "qk"), "v": ("wo", "qk", "v"), "wo": ("qk", "v", "wo"),
                   None: ("qk", "v", "wo")}[last]
            c = [x for x in rot if x in cand][0]
            last = c
            if c == "qk":
                out.append(("qk", nqk)); t += dur_qk; qk_end[nqk] = t; nqk += 1
            elif c == "v":
                out.append(("v", nv)); t += dur_v[nv]; v_end[nv] = t; nv += 1
            else:
                out.append(("wo", nwo)); t += 40; nwo += 1
    return out


def _kernel(x_hbm, mem0_ref, wq_hbm, wk_hbm, wv_hbm, wo_hbm, wr_ref, wg_hbm, wu_hbm, wd_hbm,
            out_hbm,
            x_ref, xs_ref, xp_scr, raw_scr, w_ref, wo_ref, wg_ref, wu_ref, wd_ref,
            pre_scr, xn_scr, xa_scr, xc_scr, xb_scr, ot_scr, pin_scr, out_v, sems,
            *, S, D, H, DH, M, F):
    L = M + SEG
    L0 = L - PR
    nseg = S // SEG
    nblk = nseg // U
    HP = H // 2
    NC = D // DH
    NF = F // DH
    NFH = NFILL * (U - 1)
    fill_heads = list(range(H - NFH, H))
    scale = float(np.asarray(DH ** -0.5).astype(BF16))

    NXC = 4
    xc = nseg // NXC
    sem_xs, sem_x, sem_o, sem_o2, sem_xb = 0, NXC, NXC + 1, NXC + 2, NXC + 3
    sem_w = NXC + 4
    sem_wo = sem_w + 3 * HP
    sem_ffn = sem_wo + NC

    for c in range(NXC):
        pltpu.make_async_copy(x_hbm.at[c * xc:(c + 1) * xc, SEG - PR:SEG, :],
                              xs_ref.at[c * xc:(c + 1) * xc], sems.at[sem_xs + c]).start()
    XA = U + 1
    cp_xa = pltpu.make_async_copy(x_hbm.at[0:XA], x_ref.at[0:XA], sems.at[sem_x])
    cp_xb = pltpu.make_async_copy(x_hbm.at[XA:nseg], x_ref.at[XA:nseg], sems.at[sem_xb])
    X_AFTER = _env("X_AFTER", 30)
    for wi, w_hbm in enumerate((wq_hbm, wk_hbm, wv_hbm)):
        w32 = w_hbm.bitcast(U32)
        for j in range(HP):
            i = wi * HP + j
            pltpu.make_async_copy(w32.at[:, j, :], raw_scr.at[i], sems.at[sem_w + i]).start()
            if i == X_AFTER:
                cp_xa.start()
    wo_cps = [pltpu.make_async_copy(wo_hbm.bitcast(U32).at[:, c * DH:(c + 1) * DH], wo_ref.at[c],
                                    sems.at[sem_wo + c]) for c in range(NC)]
    for cp in wo_cps:
        cp.start()
    cp_xb.start()

    def wait_raw(i):
        pltpu.make_async_copy(raw_scr.at[i], raw_scr.at[i], sems.at[sem_w + i]).wait()

    def unpack(i):
        for cb in range(D // 128):
            a = raw_scr[i, pl.ds(cb * 128, 64, stride=2), :]
            b = raw_scr[i, pl.ds(cb * 128 + 1, 64, stride=2), :]
            w_ref[2 * i, cb * 64:(cb + 1) * 64, :] = (a & jnp.uint32(0xFFFF)) | (b << 16)
            w_ref[2 * i + 1, cb * 64:(cb + 1) * 64, :] = (a >> 16) | (b & jnp.uint32(0xFFFF0000))

    def sel_rows(base, seg0):
        parts = []
        for u in range(U):
            r = _mult(base + (seg0 + u) * SEG + (SEG - PR), PR)
            parts.append(xn_scr[pl.ds(r, PR), :])
        return jnp.concatenate(parts, axis=0)

    def fill(i, lhs, prow):
        pre_scr[2 * H + i, pl.ds(prow, U * PR), :] = _dot(lhs, _w(w_ref[2 * H + fill_heads[i]]))

    def ln_sel(c, carry):
        blk = xs_ref.at[pl.ds(c * xc, xc)]
        pltpu.make_async_copy(blk, blk, sems.at[sem_xs + c]).wait()
        xv = xs_ref[pl.ds(c * xc, xc)].astype(F32).reshape(xc * PR, D)
        xp_scr[pl.ds(pl.multiple_of(c * xc * PR, xc * PR), xc * PR), :] = _ln(xv).astype(BF16)
        return carry

    with _scope('p_ln'):
        lax.fori_loop(0, NXC, ln_sel, 0)
        pin_scr[...] = jnp.zeros_like(pin_scr)
        wait_raw(0)
        unpack(0)

    HI = 4
    NI = H // HI
    UP = 3

    def pre_iter(hd0, nh, pairs):
        for i in pairs:
            wait_raw(i)
        xp = xp_scr[0:nseg * PR, :]
        pairs = list(pairs)
        for e in range(nh):
            pre_scr[hd0 + e, 0:nseg * PR, :] = _dot(xp, _w(w_ref[hd0 + e]))
            if e < nh - 1:
                take = -(-len(pairs) // (nh - 1 - e))
                for i in pairs[:take]:
                    unpack(i)
                pairs = pairs[take:]

    def pre_qk(it, carry):
        pre_iter(HI * it, HI, [UP * it + 1 + e for e in range(UP)])
        return carry

    with _scope('p_0'):
        pre_iter(0, 2, [1])
        pre_iter(2, 2, [2, 3])
    with _scope('p_qk'):
        lax.fori_loop(1, 2 * NI - 1, pre_qk, 0)
    with _scope('p_last'):
        cp_xa.wait()
        pre_iter(HI * (2 * NI - 1), HI, list(range(UP * (2 * NI - 1) + 1, 3 * HP)))
        xn_scr[0:SEG, :] = _ln(x_ref[0].astype(F32))
        lhs0 = xp_scr[0:U * PR, :]
        for i in range(NFH):
            fill(i, lhs0, 0)
    with _scope('w_wo'):
        for cp in wo_cps:
            cp.wait()
    ffn_cps = []
    for src, dst, nb in ((wg_hbm, wg_ref, NF), (wu_hbm, wu_ref, NF), (wd_hbm, wd_ref, NC)):
        for c in range(nb):
            ffn_cps.append(pltpu.make_async_copy(src.bitcast(U32).at[:, c * DH:(c + 1) * DH], dst.at[c],
                                                 sems.at[sem_ffn + len(ffn_cps)]))
            ffn_cps[-1].start()

    row = lax.broadcasted_iota(jnp.int32, (L, L), 0)
    col = lax.broadcasted_iota(jnp.int32, (L, L), 1)
    mask = (row < M) | (row >= col)
    wr = wr_ref[...].astype(F32).reshape(1, D)
    OB = U * SEG

    def out_copy(r0, nrows, sem):
        return pltpu.make_async_copy(out_v.at[pl.ds(r0, nrows)], out_hbm.at[pl.ds(r0, nrows)], sems.at[sem])

    def layer(li):
        base = li * S
        first = li == 0
        dur_v = [32 if hd in fill_heads else 40 for hd in range(H)]
        sfx = "1" if first else "2"
        order = _step_order(H, 64 if first else 80, dur_v,
                            _env("LEAD" + sfx, 8 if first else 32), _env("HOLD" + sfx, 9),
                            _env("FIN" + sfx, 1200), _env("LMM", 155), _env("LSM", 330))

        def finish(sp, o_tok, best_v, best_s, valid):
            r0 = _mult(sp * SEG, SEG)
            xin = x_ref[sp].astype(F32) if first else xb_scr[pl.ds(r0, SEG), :]
            x1 = _rb(xin + o_tok)
            xn1 = _ln(x1)
            r = _rb(jnp.sum(xn1 * wr, axis=-1, keepdims=True))
            upd = r > best_v
            if valid is not None:
                upd = jnp.logical_and(upd, valid)
            best_v = jnp.where(upd, r, best_v)
            best_s = jnp.where(upd, sp, best_s)
            x2 = _rb(x1 + xn1)
            xa_scr[pl.ds(r0, SEG), :] = x1
            if first:
                xc_scr[pl.ds(r0, SEG), :] = xn1
                xb_scr[pl.ds(r0, SEG), :] = x2
                xn_scr[pl.ds(S + r0, SEG), :] = _ln(x2)
            else:
                xn_scr[pl.ds(r0, SEG), :] = xn1
                out_v[pl.ds(r0, SEG), :] = x2.astype(BF16)
            return best_v, best_s

        def segment(s, mem, prev_tok, best_v, best_s, valid):
            r0 = pl.multiple_of(base + s * SEG, SEG)
            p0 = pl.multiple_of(s * PR, PR)
            hh = [jnp.concatenate([mem, xn_scr[pl.ds(r0, SEG), :]], axis=0)]
            q = [None] * H
            k = [None] * H
            v = [None] * H
            p = [None] * H
            il = [None] * H
            o = [None] * H
            dd = [None] * H
            acc = None
            nacc = 0
            za = pl.multiple_of((s >> 12) * 8, 8)
            zb = pl.multiple_of((s >> 13) * 8, 8)

            def proj(wi, pcol):
                if pcol is None:
                    return _dot(hh[0], _w(w_ref[wi]))
                return jnp.concatenate(
                    [_dot(hh[0][:L0], _w(w_ref[wi])), pre_scr[pcol, pl.ds(p0, PR), :]], axis=0)

            for kind, i in order:
                if kind == "qk":
                    q[i] = proj(i, i if first else None)
                    k[i] = proj(H + i, H + i if first else None)
                elif kind == "s":
                    for hd in range(i * G, (i + 1) * G):
                        sc = _dot_nt(q[hd], k[hd]) * scale
                        sc = jnp.where(mask, sc, -1e9)
                        mx = jnp.max(sc, axis=-1, keepdims=True)
                        e = jnp.exp(sc - mx)
                        p[hd] = e
                        il[hd] = pl.reciprocal(jnp.sum(e, axis=-1, keepdims=True), approx=True)
                elif kind == "v":
                    v[i] = proj(2 * H + i, 2 * H + fill_heads.index(i) if i in fill_heads else None)
                elif kind == "pv":
                    for hd in range(i * G, (i + 1) * G):
                        o[hd] = _dot(p[hd], v[hd]) * il[hd]
                elif kind == "wo":
                    lhs = o[i]
                    if i - PIN_GAP in PIN_AT:
                        z = pin_scr[pl.ds(zb, 8), 0:DH]
                        lhs = jnp.concatenate([lhs[:8] + z, lhs[8:]], axis=0)
                    dd[i] = jnp.concatenate(
                        [_dot(lhs, _w(wo_ref[c, i * (DH // 2):(i + 1) * (DH // 2), :])) for c in range(NC)],
                        axis=1)
                    if i in PIN_AT:
                        while nacc <= i - PIN_LAG:
                            acc = dd[nacc] if acc is None else acc + dd[nacc]
                            nacc += 1
                        pin_scr[pl.ds(za + 8, L), :] = acc
                elif kind == "finish":
                    sp = s - 1 if valid is None else jnp.maximum(s - 1, 0)
                    best_v, best_s = finish(sp, prev_tok, best_v, best_s, valid)
                    if first:
                        sn = jnp.minimum(s + 1, nseg - 1)
                        xn_scr[pl.ds(pl.multiple_of(sn * SEG, SEG), SEG), :] = _ln(x_ref[sn].astype(F32))
                    hh[0] = jnp.concatenate([mem, xn_scr[pl.ds(r0, SEG), :]], axis=0)
            for j in range(nacc, H):
                acc = acc + dd[j]
            res = _rb(acc)
            return res[:M], res[M:], best_v, best_s

        def block(b, carry):
            mem, best_v, best_s = carry
            if first:
                @pl.when(b == 1)
                def _():
                    cp_xb.wait()
            else:
                @pl.when(b >= 2)
                def _():
                    out_copy(pl.multiple_of((b - 2) * OB, OB), OB, sem_o).start()
            tok = ot_scr[...]
            nb = jnp.minimum(b + 1, nblk - 1)
            for u in range(U):
                s = b * U + u
                mem, tok, best_v, best_s = segment(s, mem, tok, best_v, best_s, (s > 0) if u == 0 else None)
                if u < U - 1:
                    if first:
                        lhs = xp_scr[pl.ds(pl.multiple_of(nb * U * PR, U * PR), U * PR), :]
                    else:
                        lhs = sel_rows(base, nb * U)
                    for i in range(u * NFILL, (u + 1) * NFILL):
                        fill(i, lhs, pl.multiple_of((b + 1) * U * PR, U * PR))
            ot_scr[...] = tok
            return mem, best_v, best_s

        ot_scr[...] = jnp.zeros_like(ot_scr)
        init = (mem0_ref[...].astype(F32),
                jnp.full((SEG, 1), -jnp.inf, F32),
                jnp.zeros((SEG, 1), jnp.int32))
        with _scope('main%d' % li):
            _, best_v, best_s = lax.fori_loop(0, nblk, block, init)
        best_v, best_s = finish(nseg - 1, ot_scr[...], best_v, best_s, None)
        if first:
            for cp in ffn_cps:
                cp.wait()
        else:
            out_copy((nblk - 2) * OB, 2 * OB, sem_o).start()

        vmax = jnp.max(best_v, axis=0, keepdims=True)
        tok = best_s * SEG + lax.broadcasted_iota(jnp.int32, (SEG, 1), 0)
        idx = jnp.min(jnp.where(best_v == vmax, tok, S))
        idx = jnp.clip(idx, 0, S - 1)
        xs = xc_scr[pl.ds(idx, 1), :] if first else xn_scr[pl.ds(idx, 1), :]
        x1 = xa_scr[pl.ds(idx, 1), :]
        xs8 = jnp.broadcast_to(xs, (8, D))
        g = _rb(jnp.concatenate([_dot(xs8, _w(wg_ref[c])) for c in range(NF)], axis=1))
        u = _rb(jnp.concatenate([_dot(xs8, _w(wu_ref[c])) for c in range(NF)], axis=1))
        g = _rb(g * _rb(jax.nn.sigmoid(g)))
        gu = _rb(g * u)
        y = _rb(jnp.concatenate([_dot(gu, _w(wd_ref[c])) for c in range(NC)], axis=1))
        y = _rb(y * _rb(jax.nn.sigmoid(vmax)))
        new = _rb(x1 + _rb(xs + y[0:1]))
        return idx, new

    idx, new = layer(0)
    xb_scr[pl.ds(idx, 1), :] = new
    xn_scr[pl.ds(S + idx, 1), :] = _ln(new)
    lhs0 = sel_rows(S, 0)
    for i in range(NFH):
        fill(i, lhs0, 0)

    idx, new = layer(1)
    out_copy(0, S, sem_o).wait()
    b0 = pl.multiple_of((idx // 16) * 16, 16)
    blk = out_v[pl.ds(b0, 16), :].astype(F32)
    rid = b0 + lax.broadcasted_iota(jnp.int32, (16, D), 0)
    out_v[pl.ds(b0, 16), :] = jnp.where(rid == idx, new, blk).astype(BF16)
    cp = out_copy(b0, 16, sem_o2)
    cp.start()
    cp.wait()


@jax.jit
def pallas_interleave_layers__memory_aug_recurrent_mem_tr__moe_arch_mod__prompt_kernel(
    A_x, A_mem0, A_Wq, A_Wk, A_Wv, A_Wo, A_seg_len, B_x, B_w_r, B_w_gate, B_w_up, B_w_down,
):
    B, S, D = A_x.shape
    _, H, DH = A_Wq.shape
    M = A_mem0.shape[1]
    F = B_w_gate.shape[1]
    assert B == 1 and S % (SEG * U) == 0
    nseg = S // SEG
    kern = functools.partial(_kernel, S=S, D=D, H=H, DH=DH, M=M, F=F)
    hbm = pl.BlockSpec(memory_space=pl.ANY)
    vm = pl.BlockSpec(memory_space=pltpu.VMEM)
    nsem = 8 + 3 * (H // 2) + D // DH + 2 * (F // DH) + D // DH
    out = pl.pallas_call(
        kern,
        out_shape=jax.ShapeDtypeStruct((S, D), BF16),
        in_specs=[hbm, vm, hbm, hbm, hbm, hbm, vm, hbm, hbm, hbm],
        out_specs=hbm,
        scratch_shapes=[
            pltpu.VMEM((nseg, SEG, D), BF16),
            pltpu.VMEM((nseg, PR, D), BF16),
            pltpu.VMEM((nseg * PR, D), BF16),
            pltpu.VMEM((3 * (H // 2), D, DH), U32),
            pltpu.VMEM((3 * H, D // 2, DH), U32),
            pltpu.VMEM((D // DH, H * DH // 2, DH), U32),
            pltpu.VMEM((F // DH, D // 2, DH), U32), pltpu.VMEM((F // DH, D // 2, DH), U32),
            pltpu.VMEM((D // DH, F // 2, DH), U32),
            pltpu.VMEM((2 * H + NFILL * (U - 1), (nseg + U) * PR, DH), F32),
            pltpu.VMEM((2 * S, D), F32),
            pltpu.VMEM((S, D), F32), pltpu.VMEM((S, D), F32), pltpu.VMEM((S, D), F32),
            pltpu.VMEM((SEG, D), F32),
            pltpu.VMEM((M + SEG + 8, D), F32),
            pltpu.VMEM((S, D), BF16),
            pltpu.SemaphoreType.DMA((nsem,))],
        compiler_params=pltpu.CompilerParams(vmem_limit_bytes=110 * 1024 * 1024),
    )(A_x.reshape(nseg, SEG, D), A_mem0.reshape(M, D), A_Wq, A_Wk, A_Wv,
      A_Wo.reshape(H * DH, D), B_w_r, B_w_gate, B_w_up, B_w_down)
    return out.reshape(B, S, D)
```

```python
import functools
import numpy as np
import jax
import jax.numpy as jnp
from jax import lax
import jax.experimental.pallas as pl
import jax.experimental.pallas.tpu as pltpu

F32 = jnp.float32
BF16 = jnp.bfloat16
U32 = jnp.uint32
SEG = 32
EPS = 1e-05
G = 4
PR = 8


def _env(name, default):
    return default


U = _env("U", 4)
NFILL = _env("NFILL", 5)
PIN_LAG = _env("PIN_LAG", 4)
PIN_GAP = _env("PIN_GAP", 2)
PIN_AT = [int(t) for t in "4,6,8,10,12,14,16,18,20,22,24,26,28,29".split(",")]
NVB = _env("NVB", 1)
VB2 = [int(t) for t in "".split(",") if t]
PPIN = _env("PPIN", 0) == 1
KS = _env("KS", 2)
LOG2E = 1.4426950408889634
SCOPES = _env("SCOPES", 0)


class _NoScope:
    def __enter__(self):
        return self

    def __exit__(self, *a):
        return False


def _scope(name):
    return jax.named_scope(name) if SCOPES else _NoScope()


def _rb(x):
    return x.astype(BF16).astype(F32)


def _ln(x):
    d = x.shape[-1]
    mu = jnp.sum(x, axis=-1, keepdims=True) * (1.0 / d)
    c = x - mu
    var = jnp.sum(c * c, axis=-1, keepdims=True) * (1.0 / d)
    m = _rb(mu)
    v = _rb(var)
    den = _rb(jnp.sqrt(_rb(v + EPS)))
    return _rb(_rb(x - m) / den)


def _w(x):
    return pltpu.bitcast(x, BF16)


def _dot(a, b):
    return lax.dot_general(a, b, (((1,), (0,)), ((), ())), preferred_element_type=F32)


def _dot_nt(a, b):
    return lax.dot_general(a, b, (((1,), (1,)), ((), ())), preferred_element_type=F32)


def _tree(f, xs):
    xs = list(xs)
    while len(xs) > 1:
        xs = [f(xs[i], xs[i + 1]) if i + 1 < len(xs) else xs[i] for i in range(0, len(xs), 2)]
    return xs[0]


def _mult(r, m):
    return r if isinstance(r, int) else pl.multiple_of(r, m)


def _step_order(H, dur_qk, dur_v, dur_a, lead, hold, fin_at, l_mm, l_sm, l_pin):
    NG = H // G
    out = []
    t = 0
    nqk = nv = nwo = ns = npv = 0
    qk_end = [0] * H
    v_end = [0] * H
    s_end = [0] * NG
    pv_end = [0] * NG
    last = None
    fin_done = False
    npin = 0
    while nwo < H:
        if not fin_done and t >= fin_at:
            out.append(("finish", 0))
            fin_done = True
        s_ok = ns < NG and nqk >= (ns + 1) * G and t >= qk_end[(ns + 1) * G - 1] + l_mm
        pv_ok = (npv < ns and nv >= (npv + 1) * G and t >= v_end[(npv + 1) * G - 1] + l_mm
                 and t >= s_end[npv] + l_sm)
        qk_ok = nqk < H
        v_ok = nv < H and (nqk >= H or nv + lead < nqk)
        wo_ok = (nwo < npv * G and t >= pv_end[nwo // G] + l_mm and (nv >= H or nwo + hold < nv))
        if s_ok:
            out.append(("s", ns)); t += dur_a[ns]; s_end[ns] = t; ns += 1
        elif pv_ok:
            out.append(("pv", npv)); t += dur_a[npv]; pv_end[npv] = t; npv += 1
        else:
            cand = [c for c, ok in (("qk", qk_ok), ("v", v_ok), ("wo", wo_ok)) if ok]
            if not cand:
                t += 4
                continue
            rot = {"qk": ("v", "wo", "qk"), "v": ("wo", "qk", "v"), "wo": ("qk", "v", "wo"),
                   None: ("qk", "v", "wo")}[last]
            c = [x for x in rot if x in cand][0]
            last = c
            if c in ("qk", "v") and npin < ns and t >= s_end[npin] + l_pin:
                while npin < ns and t >= s_end[npin] + l_pin:
                    out.append(("ppin", npin))
                    npin += 1
            if c == "qk":
                out.append(("qk", nqk)); t += dur_qk[nqk]; qk_end[nqk] = t; nqk += 1
            elif c == "v":
                out.append(("v", nv)); t += dur_v[nv]; v_end[nv] = t; nv += 1
            else:
                out.append(("wo", nwo)); t += 40; nwo += 1
    return out


def _kernel(x_hbm, mem0_ref, wq_hbm, wk_hbm, wv_hbm, wo_hbm, wr_ref, wg_hbm, wu_hbm, wd_hbm,
            out_hbm,
            x_ref, xs_ref, xp_scr, raw_scr, w_ref, wo_ref, wg_ref, wu_ref, wd_ref,
            pre_scr, xn_scr, xa_scr, xc_scr, xb_scr, ot_scr, pin_scr, out_v, ks_scr, vs_scr, pin2_scr, p_scr, sems,
            *, S, D, H, DH, M, F):
    L = M + SEG
    L0 = L - PR
    nseg = S // SEG
    nblk = nseg // U
    HP = H // 2
    NC = D // DH
    NF = F // DH
    NFH = NFILL * (U - 1)
    fill_heads = list(range(H - NFH, H))
    scale = float(np.asarray(DH ** -0.5).astype(BF16))
    nvb = [NVB + (1 if (hd // G) in VB2 else 0) for hd in range(H)]
    KR = M + 8 * max(nvb)

    NXC = 4
    xc = nseg // NXC
    sem_xs, sem_x, sem_o, sem_o2, sem_xb = 0, NXC, NXC + 1, NXC + 2, NXC + 3
    sem_w = NXC + 4
    sem_wo = sem_w + 3 * HP
    sem_ffn = sem_wo + NC

    for c in range(NXC):
        pltpu.make_async_copy(x_hbm.at[c * xc:(c + 1) * xc, SEG - PR:SEG, :],
                              xs_ref.at[c * xc:(c + 1) * xc], sems.at[sem_xs + c]).start()
    XA = U + 1
    cp_xa = pltpu.make_async_copy(x_hbm.at[0:XA], x_ref.at[0:XA], sems.at[sem_x])
    cp_xb = pltpu.make_async_copy(x_hbm.at[XA:nseg], x_ref.at[XA:nseg], sems.at[sem_xb])
    X_AFTER = _env("X_AFTER", 30)
    for wi, w_hbm in enumerate((wq_hbm, wk_hbm, wv_hbm)):
        w32 = w_hbm.bitcast(U32)
        for j in range(HP):
            i = wi * HP + j
            pltpu.make_async_copy(w32.at[:, j, :], raw_scr.at[i], sems.at[sem_w + i]).start()
            if i == X_AFTER:
                cp_xa.start()
    wo_cps = [pltpu.make_async_copy(wo_hbm.bitcast(U32).at[:, c * DH:(c + 1) * DH], wo_ref.at[c],
                                    sems.at[sem_wo + c]) for c in range(NC)]
    for cp in wo_cps:
        cp.start()
    cp_xb.start()

    def wait_raw(i):
        pltpu.make_async_copy(raw_scr.at[i], raw_scr.at[i], sems.at[sem_w + i]).wait()

    def unpack(i):
        for cb in range(D // 128):
            a = raw_scr[i, pl.ds(cb * 128, 64, stride=2), :]
            b = raw_scr[i, pl.ds(cb * 128 + 1, 64, stride=2), :]
            w_ref[2 * i, cb * 64:(cb + 1) * 64, :] = (a & jnp.uint32(0xFFFF)) | (b << 16)
            w_ref[2 * i + 1, cb * 64:(cb + 1) * 64, :] = (a >> 16) | (b & jnp.uint32(0xFFFF0000))

    def sel_rows(base, seg0):
        parts = []
        for u in range(U):
            r = _mult(base + (seg0 + u) * SEG + (SEG - PR), PR)
            parts.append(xn_scr[pl.ds(r, PR), :])
        return jnp.concatenate(parts, axis=0)

    def fill(i, lhs, prow):
        pre_scr[2 * H + i, pl.ds(prow, U * PR), :] = _dot(lhs, _w(w_ref[2 * H + fill_heads[i]]))

    def ln_sel(c, carry):
        blk = xs_ref.at[pl.ds(c * xc, xc)]
        pltpu.make_async_copy(blk, blk, sems.at[sem_xs + c]).wait()
        xv = xs_ref[pl.ds(c * xc, xc)].astype(F32).reshape(xc * PR, D)
        xp_scr[pl.ds(pl.multiple_of(c * xc * PR, xc * PR), xc * PR), :] = _ln(xv).astype(BF16)
        return carry

    with _scope('p_ln'):
        lax.fori_loop(0, NXC, ln_sel, 0)
        pin_scr[...] = jnp.zeros_like(pin_scr)
        pin2_scr[...] = jnp.zeros_like(pin2_scr)
        p_scr[0:8, :] = jnp.zeros((8, DH), F32)
        for scr in (ks_scr, vs_scr):
            if VB2:
                scr[...] = jnp.zeros_like(scr)
            else:
                scr[0:8, :] = jnp.zeros((8, DH), F32)
        wait_raw(0)
        unpack(0)

    HI = 4
    NI = H // HI
    UP = 3

    def pre_wi(slot):
        nk = H // KS
        if isinstance(slot, int):
            return slot if slot < H else (H + KS * (slot - H) if slot < H + nk else 2 * H + slot - H - nk)
        return jnp.where(slot < H, slot, jnp.where(slot < H + nk, H + KS * (slot - H), H + slot - nk))

    pre_slot = {pre_wi(t): t for t in range(2 * H)}

    def pre_iter(hd0, nh, pairs):
        for i in pairs:
            wait_raw(i)
        xp = xp_scr[0:nseg * PR, :]
        pairs = list(pairs)
        for e in range(nh):
            pre_scr[hd0 + e, 0:nseg * PR, :] = _dot(xp, _w(w_ref[pre_wi(hd0 + e)]))
            if e < nh - 1:
                take = -(-len(pairs) // (nh - 1 - e))
                for i in pairs[:take]:
                    unpack(i)
                pairs = pairs[take:]

    def pre_qk(it, carry):
        pre_iter(HI * it, HI, [UP * it + 1 + e for e in range(UP)])
        return carry

    with _scope('p_0'):
        pre_iter(0, 2, [1])
        pre_iter(2, 2, [2, 3])
    with _scope('p_qk'):
        lax.fori_loop(1, 2 * NI - 1, pre_qk, 0)
    with _scope('p_last'):
        cp_xa.wait()
        pre_iter(HI * (2 * NI - 1), HI, list(range(UP * (2 * NI - 1) + 1, 3 * HP)))
        xn_scr[0:SEG, :] = _ln(x_ref[0].astype(F32))
        lhs0 = xp_scr[0:U * PR, :]
        for i in range(NFH):
            fill(i, lhs0, 0)
    with _scope('w_wo'):
        for cp in wo_cps:
            cp.wait()
    ffn_cps = []
    for src, dst, nb in ((wg_hbm, wg_ref, NF), (wu_hbm, wu_ref, NF), (wd_hbm, wd_ref, NC)):
        for c in range(nb):
            ffn_cps.append(pltpu.make_async_copy(src.bitcast(U32).at[:, c * DH:(c + 1) * DH], dst.at[c],
                                                 sems.at[sem_ffn + len(ffn_cps)]))
            ffn_cps[-1].start()

    row = lax.broadcasted_iota(jnp.int32, (L, L), 0)
    col = lax.broadcasted_iota(jnp.int32, (L, L), 1)
    mask = (row < M) | (row >= col)
    wr = wr_ref[...].astype(F32).reshape(1, D)
    masks = {}
    for nb_ in set(nvb) - {0}:
        rr = lax.broadcasted_iota(jnp.int32, (L - 8 * nb_, L), 0)
        cc = lax.broadcasted_iota(jnp.int32, (L - 8 * nb_, L), 1)
        masks[nb_] = (rr < M) | (rr + 8 * nb_ >= cc)
    row8 = lax.broadcasted_iota(jnp.int32, (8, DH), 0)

    def vpu_scores(hd, j, qb):
        b0 = 8 + KR * hd
        qs = qb * (scale * LOG2E)
        ss = []
        for o_ in range(-7, M + 8 * j + 1):
            sv = jnp.sum(qs * ks_scr[b0 + o_:b0 + o_ + 8, :], axis=-1, keepdims=True)
            sv = jnp.broadcast_to(sv, (8, DH))
            if o_ < 0:
                sv = jnp.where(row8 >= -o_, sv, -1e9 * LOG2E)
            ss.append(sv)
        mx = _tree(jnp.maximum, ss)
        return [jnp.exp2(sv - mx) for sv in ss]

    def vpu_pv(hd, j, ps):
        b0 = 8 + KR * hd
        offs = range(-7, M + 8 * j + 1)
        den = _tree(jnp.add, ps)
        acc = _tree(jnp.add, [pv * vs_scr[b0 + o_:b0 + o_ + 8, :] for pv, o_ in zip(ps, offs)])
        return acc * pl.reciprocal(den, approx=True)

    OB = U * SEG

    def out_copy(r0, nrows, sem):
        return pltpu.make_async_copy(out_v.at[pl.ds(r0, nrows)], out_hbm.at[pl.ds(r0, nrows)], sems.at[sem])

    def layer(li):
        base = li * S
        first = li == 0
        dur_v = [32 if (hd in fill_heads or (first and 2 * H + hd in pre_slot)) else 40 for hd in range(H)]
        dur_qk = [(32 + (32 if H + hd in pre_slot else 40)) if first else 80 for hd in range(H)]
        sfx = "1" if first else "2"
        order = _step_order(H, dur_qk, dur_v, [L - 8 * nvb[g * G] for g in range(H // G)],
                            _env("LEAD" + sfx, 32), _env("HOLD" + sfx, 9),
                            _env("FIN" + sfx, 2600 if first else 1200), _env("LMM", 155), _env("LSM", 450), _env("LPIN", 450))

        voff = _env("VOFF" + sfx, 32)

        def finish(sp, o_tok, best_v, best_s, valid):
            r0 = _mult(sp * SEG, SEG)
            xin = x_ref[sp].astype(F32) if first else xb_scr[pl.ds(r0, SEG), :]
            x1 = _rb(xin + o_tok)
            xn1 = _ln(x1)
            r = _rb(jnp.sum(xn1 * wr, axis=-1, keepdims=True))
            upd = r > best_v
            if valid is not None:
                upd = jnp.logical_and(upd, valid)
            best_v = jnp.where(upd, r, best_v)
            best_s = jnp.where(upd, sp, best_s)
            x2 = _rb(x1 + xn1)
            xa_scr[pl.ds(r0, SEG), :] = x1
            if first:
                xc_scr[pl.ds(r0, SEG), :] = xn1
                xb_scr[pl.ds(r0, SEG), :] = x2
                xn_scr[pl.ds(S + r0, SEG), :] = _ln(x2)
            else:
                xn_scr[pl.ds(r0, SEG), :] = xn1
                out_v[pl.ds(r0, SEG), :] = x2.astype(BF16)
            return best_v, best_s

        def segment(s, mem, prev_tok, best_v, best_s, valid):
            r0 = pl.multiple_of(base + s * SEG, SEG)
            p0 = pl.multiple_of(s * PR, PR)
            hh = [jnp.concatenate([mem, xn_scr[pl.ds(r0, SEG), :]], axis=0)]
            q = [None] * H
            k = [None] * H
            v = [None] * H
            p = [None] * H
            il = [None] * H
            o = [None] * H
            dd = [None] * H
            pw = [None] * H
            acc = None
            nacc = 0
            za = pl.multiple_of((s >> 12) * 8, 8)
            zb = pl.multiple_of((s >> 13) * 8, 8)

            ppin = [False]

            def proj(wi, pcol):
                lhs = hh[0]
                if ppin[0]:
                    ppin[0] = False
                    z = p_scr[0:8, :]
                    top = jnp.concatenate([lhs[:8, :DH] + z, lhs[:8, DH:]], axis=1)
                    lhs = jnp.concatenate([top, lhs[8:]], axis=0)
                if pcol is None:
                    return _dot(lhs, _w(w_ref[wi]))
                return jnp.concatenate(
                    [_dot(lhs[:L0], _w(w_ref[wi])), pre_scr[pcol, pl.ds(p0, PR), :]], axis=0)

            for kind, i in order:
                if kind == "qk":
                    q[i] = proj(i, i if first else None)
                    k[i] = proj(H + i, pre_slot.get(H + i) if first else None)
                    if nvb[i]:
                        nk = M + 8 * nvb[i]
                        ks_scr[8 + KR * i:8 + KR * i + nk, :] = k[i][:nk]
                elif kind == "s":
                    for hd in range(i * G, (i + 1) * G):
                        qm = q[hd]
                        mk = mask
                        if nvb[hd]:
                            qm = jnp.concatenate([qm[:M], qm[M + 8 * nvb[hd]:]], axis=0)
                            mk = masks[nvb[hd]]
                        sc = _dot_nt(qm, k[hd]) * scale
                        sc = jnp.where(mk, sc, -1e9)
                        mx = jnp.max(sc, axis=-1, keepdims=True)
                        e = jnp.exp(sc - mx)
                        pn = e * pl.reciprocal(jnp.sum(e, axis=-1, keepdims=True), approx=True)
                        p[hd] = pn
                elif kind == "ppin":
                    if PPIN and p[i * G] is not None:
                        for hd in range(i * G, (i + 1) * G):
                            p_scr[pl.ds(za + 8 + hd * L, p[hd].shape[0]), 0:L] = p[hd]
                            p[hd] = None
                        ppin[0] = True
                elif kind == "v":
                    v[i] = proj(2 * H + i, 2 * H + fill_heads.index(i) if i in fill_heads
                                else (pre_slot.get(2 * H + i) if first else None))
                    if nvb[i]:
                        nk = M + 8 * nvb[i]
                        vs_scr[8 + KR * i:8 + KR * i + nk, :] = v[i][:nk]
                    hd = i + voff
                    if hd < H and nvb[hd]:
                        pin2_scr[pl.ds(za + 8, 8), :] = v[i][:8]
                        z = pin2_scr[pl.ds(zb, 8), :]
                        pw[hd] = [vpu_scores(hd, j, q[hd][M + 8 * j:M + 8 * (j + 1)] + z) for j in range(nvb[hd])]
                elif kind == "pv":
                    for hd in range(i * G, (i + 1) * G):
                        if p[hd] is None:
                            p[hd] = p_scr[8 + hd * L:8 + hd * L + L - 8 * nvb[hd], 0:L]
                        om = _dot(p[hd], v[hd])
                        p[hd] = None
                        if nvb[hd]:
                            if pw[hd] is None:
                                pw[hd] = [vpu_scores(hd, j, q[hd][M + 8 * j:M + 8 * (j + 1)]) for j in range(nvb[hd])]
                            ov = [vpu_pv(hd, j, pw[hd][j]) for j in range(nvb[hd])]
                            om = jnp.concatenate([om[:M]] + ov + [om[M:]], axis=0)
                        o[hd] = om
                elif kind == "wo":
                    lhs = o[i]
                    if i - PIN_GAP in PIN_AT:
                        z = pin_scr[pl.ds(zb, 8), 0:DH]
                        lhs = jnp.concatenate([lhs[:8] + z, lhs[8:]], axis=0)
                    dd[i] = jnp.concatenate(
                        [_dot(lhs, _w(wo_ref[c, i * (DH // 2):(i + 1) * (DH // 2), :])) for c in range(NC)],
                        axis=1)
                    if i in PIN_AT:
                        while nacc <= i - PIN_LAG:
                            acc = dd[nacc] if acc is None else acc + dd[nacc]
                            nacc += 1
                        pin_scr[pl.ds(za + 8, L), :] = acc
                elif kind == "finish":
                    sp = s - 1 if valid is None else jnp.maximum(s - 1, 0)
                    best_v, best_s = finish(sp, prev_tok, best_v, best_s, valid)
                    if first:
                        sn = jnp.minimum(s + 1, nseg - 1)
                        xn_scr[pl.ds(pl.multiple_of(sn * SEG, SEG), SEG), :] = _ln(x_ref[sn].astype(F32))
                    hh[0] = jnp.concatenate([mem, xn_scr[pl.ds(r0, SEG), :]], axis=0)
            for j in range(nacc, H):
                acc = acc + dd[j]
            res = _rb(acc)
            return res[:M], res[M:], best_v, best_s

        def block(b, carry):
            mem, best_v, best_s = carry
            if first:
                @pl.when(b == 1)
                def _():
                    cp_xb.wait()
            else:
                @pl.when(b >= 2)
                def _():
                    out_copy(pl.multiple_of((b - 2) * OB, OB), OB, sem_o).start()
            tok = ot_scr[...]
            nb = jnp.minimum(b + 1, nblk - 1)
            for u in range(U):
                s = b * U + u
                mem, tok, best_v, best_s = segment(s, mem, tok, best_v, best_s, (s > 0) if u == 0 else None)
                if u < U - 1:
                    if first:
                        lhs = xp_scr[pl.ds(pl.multiple_of(nb * U * PR, U * PR), U * PR), :]
                    else:
                        lhs = sel_rows(base, nb * U)
                    for i in range(u * NFILL, (u + 1) * NFILL):
                        fill(i, lhs, pl.multiple_of((b + 1) * U * PR, U * PR))
            ot_scr[...] = tok
            return mem, best_v, best_s

        ot_scr[...] = jnp.zeros_like(ot_scr)
        init = (mem0_ref[...].astype(F32),
                jnp.full((SEG, 1), -jnp.inf, F32),
                jnp.zeros((SEG, 1), jnp.int32))
        with _scope('main%d' % li):
            _, best_v, best_s = lax.fori_loop(0, nblk, block, init)
        best_v, best_s = finish(nseg - 1, ot_scr[...], best_v, best_s, None)
        if first:
            for cp in ffn_cps:
                cp.wait()
        else:
            out_copy((nblk - 2) * OB, 2 * OB, sem_o).start()

        vmax = jnp.max(best_v, axis=0, keepdims=True)
        tok = best_s * SEG + lax.broadcasted_iota(jnp.int32, (SEG, 1), 0)
        idx = jnp.min(jnp.where(best_v == vmax, tok, S))
        idx = jnp.clip(idx, 0, S - 1)
        xs = xc_scr[pl.ds(idx, 1), :] if first else xn_scr[pl.ds(idx, 1), :]
        x1 = xa_scr[pl.ds(idx, 1), :]
        xs8 = jnp.broadcast_to(xs, (8, D))
        g = _rb(jnp.concatenate([_dot(xs8, _w(wg_ref[c])) for c in range(NF)], axis=1))
        u = _rb(jnp.concatenate([_dot(xs8, _w(wu_ref[c])) for c in range(NF)], axis=1))
        g = _rb(g * _rb(jax.nn.sigmoid(g)))
        gu = _rb(g * u)
        y = _rb(jnp.concatenate([_dot(gu, _w(wd_ref[c])) for c in range(NC)], axis=1))
        y = _rb(y * _rb(jax.nn.sigmoid(vmax)))
        new = _rb(x1 + _rb(xs + y[0:1]))
        return idx, new

    idx, new = layer(0)
    xb_scr[pl.ds(idx, 1), :] = new
    xn_scr[pl.ds(S + idx, 1), :] = _ln(new)
    lhs0 = sel_rows(S, 0)
    for i in range(NFH):
        fill(i, lhs0, 0)

    idx, new = layer(1)
    out_copy(0, S, sem_o).wait()
    b0 = pl.multiple_of((idx // 16) * 16, 16)
    blk = out_v[pl.ds(b0, 16), :].astype(F32)
    rid = b0 + lax.broadcasted_iota(jnp.int32, (16, D), 0)
    out_v[pl.ds(b0, 16), :] = jnp.where(rid == idx, new, blk).astype(BF16)
    cp = out_copy(b0, 16, sem_o2)
    cp.start()
    cp.wait()


@jax.jit
def pallas_interleave_layers__memory_aug_recurrent_mem_tr__moe_arch_mod__prompt_kernel(
    A_x, A_mem0, A_Wq, A_Wk, A_Wv, A_Wo, A_seg_len, B_x, B_w_r, B_w_gate, B_w_up, B_w_down,
):
    B, S, D = A_x.shape
    _, H, DH = A_Wq.shape
    M = A_mem0.shape[1]
    F = B_w_gate.shape[1]
    assert B == 1 and S % (SEG * U) == 0
    nseg = S // SEG
    kern = functools.partial(_kernel, S=S, D=D, H=H, DH=DH, M=M, F=F)
    hbm = pl.BlockSpec(memory_space=pl.ANY)
    vm = pl.BlockSpec(memory_space=pltpu.VMEM)
    nsem = 8 + 3 * (H // 2) + D // DH + 2 * (F // DH) + D // DH
    out = pl.pallas_call(
        kern,
        out_shape=jax.ShapeDtypeStruct((S, D), BF16),
        in_specs=[hbm, vm, hbm, hbm, hbm, hbm, vm, hbm, hbm, hbm],
        out_specs=hbm,
        scratch_shapes=[
            pltpu.VMEM((nseg, SEG, D), BF16),
            pltpu.VMEM((nseg, PR, D), BF16),
            pltpu.VMEM((nseg * PR, D), BF16),
            pltpu.VMEM((3 * (H // 2), D, DH), U32),
            pltpu.VMEM((3 * H, D // 2, DH), U32),
            pltpu.VMEM((D // DH, H * DH // 2, DH), U32),
            pltpu.VMEM((F // DH, D // 2, DH), U32), pltpu.VMEM((F // DH, D // 2, DH), U32),
            pltpu.VMEM((D // DH, F // 2, DH), U32),
            pltpu.VMEM((2 * H + NFILL * (U - 1), (nseg + U) * PR, DH), F32),
            pltpu.VMEM((2 * S, D), F32),
            pltpu.VMEM((S, D), F32), pltpu.VMEM((S, D), F32), pltpu.VMEM((S, D), F32),
            pltpu.VMEM((SEG, D), F32),
            pltpu.VMEM((M + SEG + 8, D), F32),
            pltpu.VMEM((S, D), BF16),
            pltpu.VMEM((8 + H * (M + 16), DH), F32), pltpu.VMEM((8 + H * (M + 16), DH), F32),
            pltpu.VMEM((16, DH), F32),
            pltpu.VMEM((8 + H * (M + SEG), DH), F32),
            pltpu.SemaphoreType.DMA((nsem,))],
        compiler_params=pltpu.CompilerParams(vmem_limit_bytes=110 * 1024 * 1024),
    )(A_x.reshape(nseg, SEG, D), A_mem0.reshape(M, D), A_Wq, A_Wk, A_Wv,
      A_Wo.reshape(H * DH, D), B_w_r, B_w_gate, B_w_up, B_w_down)
    return out.reshape(B, S, D)
```

```python
import functools
import numpy as np
import jax
import jax.numpy as jnp
from jax import lax
import jax.experimental.pallas as pl
import jax.experimental.pallas.tpu as pltpu

F32 = jnp.float32
BF16 = jnp.bfloat16
U32 = jnp.uint32
SEG = 32
EPS = 1e-05
G = 4
PR = 8


def _env(name, default):
    return default


U = _env("U", 4)
NFILL = _env("NFILL", 5)
PIN_LAG = _env("PIN_LAG", 4)
PIN_GAP = _env("PIN_GAP", 2)
PIN_AT = [int(t) for t in "4,6,8,10,12,14,16,18,20,22,24,26,28,29".split(",")]
NVB = _env("NVB", 1)
VB2 = [int(t) for t in "".split(",") if t]
PPIN = _env("PPIN", 0) == 1
KS = _env("KS", 1)
BFL = _env("BFL", 5)
CH = _env("CH", 8)
SERIAL = _env("SERIAL", 1)
LOG2E = 1.4426950408889634
SCOPES = _env("SCOPES", 0)


class _NoScope:
    def __enter__(self):
        return self

    def __exit__(self, *a):
        return False


def _scope(name):
    return jax.named_scope(name) if SCOPES else _NoScope()


def _rb(x):
    return x.astype(BF16).astype(F32)


def _ln(x):
    d = x.shape[-1]
    mu = jnp.sum(x, axis=-1, keepdims=True) * (1.0 / d)
    c = x - mu
    var = jnp.sum(c * c, axis=-1, keepdims=True) * (1.0 / d)
    m = _rb(mu)
    v = _rb(var)
    den = _rb(jnp.sqrt(_rb(v + EPS)))
    return _rb(_rb(x - m) / den)


def _w(x):
    return pltpu.bitcast(x, BF16)


def _dot(a, b):
    return lax.dot_general(a, b, (((1,), (0,)), ((), ())), preferred_element_type=F32)


def _dot_nt(a, b):
    return lax.dot_general(a, b, (((1,), (1,)), ((), ())), preferred_element_type=F32)


def _tree(f, xs):
    xs = list(xs)
    while len(xs) > 1:
        xs = [f(xs[i], xs[i + 1]) if i + 1 < len(xs) else xs[i] for i in range(0, len(xs), 2)]
    return xs[0]


def _mult(r, m):
    return r if isinstance(r, int) else pl.multiple_of(r, m)


def _step_order(H, dur_qk, dur_v, dur_a, lead, hold, fin_at, l_mm, l_sm, l_pin, vd, vgap):
    NG = H // G
    out = []
    t = 0
    nqk = nv = nwo = ns = npv = 0
    qk_end = [0] * H
    v_end = [0] * H
    s_end = [0] * NG
    pv_end = [0] * NG
    last = None
    fin_done = False
    npin = 0
    ends = {}
    while nwo < H:
        if not fin_done and t >= fin_at:
            out.append(("finish", 0))
            fin_done = True
        s_ok = ns < NG and nqk >= (ns + 1) * G and t >= qk_end[(ns + 1) * G - 1] + l_mm
        pv_ok = (npv < ns and nv >= (npv + 1) * G and t >= v_end[(npv + 1) * G - 1] + l_mm
                 and t >= s_end[npv] + l_sm)
        qk_ok = nqk < H
        v_ok = nv < H and (nqk >= H or nv + lead < nqk)
        wo_ok = (nwo < npv * G and t >= pv_end[nwo // G] + l_mm and (nv >= H or nwo + hold < nv))
        if s_ok:
            out.append(("s", ns)); t += dur_a[ns]; s_end[ns] = t; ns += 1
        elif pv_ok:
            out.append(("pv", npv)); t += dur_a[npv]; pv_end[npv] = t; npv += 1
        else:
            cand = [c for c, ok in (("qk", qk_ok), ("v", v_ok), ("wo", wo_ok)) if ok]
            if not cand:
                t += 4
                continue
            rot = {"qk": ("v", "wo", "qk"), "v": ("wo", "qk", "v"), "wo": ("qk", "v", "wo"),
                   None: ("qk", "v", "wo")}[last]
            c = [x for x in rot if x in cand][0]
            last = c
            if c in ("qk", "v") and npin < ns and t >= s_end[npin] + l_pin:
                while npin < ns and t >= s_end[npin] + l_pin:
                    out.append(("ppin", npin))
                    npin += 1
            if c == "qk":
                out.append(("qk", nqk)); t += dur_qk[nqk]; qk_end[nqk] = t; ends[("qk", nqk)] = t; nqk += 1
            elif c == "v":
                out.append(("v", nv)); t += dur_v[nv]; v_end[nv] = t; ends[("v", nv)] = t; nv += 1
            else:
                out.append(("wo", nwo)); t += 40; ends[("wo", nwo)] = t; nwo += 1
    if vd:
        tp = [0] * H
        for hd in range(H - 1, -1, -1):
            tp[hd] = ends[("wo", hd)] - 40 - vd
            if hd + 1 < H:
                tp[hd] = min(tp[hd], tp[hd + 1] - vgap[hd])
        after = {}
        for hd in range(H):
            cands = [key for key, e in ends.items() if e + 140 <= tp[hd] and e >= ends[("qk", hd)]]
            if cands:
                src = max(cands, key=lambda key: ends[key])
                after.setdefault(src, []).append(hd)
        out2 = []
        for op in out:
            out2.append(op)
            for hd in after.get(op, []):
                out2.append(("vs", (hd, op)))
        out = out2
    return out


def _kernel(x_hbm, mem0_ref, wq_hbm, wk_hbm, wv_hbm, wo_hbm, wr_ref, wg_hbm, wu_hbm, wd_hbm,
            out_hbm,
            x_ref, xs_ref, xp_scr, raw_scr, w_ref, wo_ref, wg_ref, wu_ref, wd_ref,
            pre_scr, xn_scr, xa_scr, xc_scr, xb_scr, ot_scr, pin_scr, out_v, ks_scr, vs_scr, pin2_scr, p_scr, sems,
            *, S, D, H, DH, M, F):
    L = M + SEG
    L0 = L - PR
    nseg = S // SEG
    nblk = nseg // U
    HP = H // 2
    NC = D // DH
    NF = F // DH
    NFH = NFILL * (U - 1)
    fill_heads = list(range(H - NFH, H))
    scale = float(np.asarray(DH ** -0.5).astype(BF16))
    nvb = [NVB + (1 if hd in VB2 else 0) for hd in range(H)]
    koff = [8 + sum(M + 8 * n for n in nvb[:hd]) for hd in range(H)]

    NXC = 4
    xc = nseg // NXC
    sem_xs, sem_x, sem_o, sem_o2, sem_xb = 0, NXC, NXC + 1, NXC + 2, NXC + 3
    sem_w = NXC + 4
    sem_wo = sem_w + 3 * HP
    sem_ffn = sem_wo + NC

    for c in range(NXC):
        pltpu.make_async_copy(x_hbm.at[c * xc:(c + 1) * xc, SEG - PR:SEG, :],
                              xs_ref.at[c * xc:(c + 1) * xc], sems.at[sem_xs + c]).start()
    XA = U + 1
    cp_xa = pltpu.make_async_copy(x_hbm.at[0:XA], x_ref.at[0:XA], sems.at[sem_x])
    cp_xb = pltpu.make_async_copy(x_hbm.at[XA:nseg], x_ref.at[XA:nseg], sems.at[sem_xb])
    X_AFTER = _env("X_AFTER", 30)
    for wi, w_hbm in enumerate((wq_hbm, wk_hbm, wv_hbm)):
        w32 = w_hbm.bitcast(U32)
        for j in range(HP):
            i = wi * HP + j
            pltpu.make_async_copy(w32.at[:, j, :], raw_scr.at[i], sems.at[sem_w + i]).start()
            if i == X_AFTER:
                cp_xa.start()
    wo_cps = [pltpu.make_async_copy(wo_hbm.bitcast(U32).at[:, c * DH:(c + 1) * DH], wo_ref.at[c],
                                    sems.at[sem_wo + c]) for c in range(NC)]
    for cp in wo_cps:
        cp.start()
    cp_xb.start()

    def wait_raw(i):
        pltpu.make_async_copy(raw_scr.at[i], raw_scr.at[i], sems.at[sem_w + i]).wait()

    def unpack(i):
        for cb in range(D // 128):
            a = raw_scr[i, pl.ds(cb * 128, 64, stride=2), :]
            b = raw_scr[i, pl.ds(cb * 128 + 1, 64, stride=2), :]
            w_ref[2 * i, cb * 64:(cb + 1) * 64, :] = (a & jnp.uint32(0xFFFF)) | (b << 16)
            w_ref[2 * i + 1, cb * 64:(cb + 1) * 64, :] = (a >> 16) | (b & jnp.uint32(0xFFFF0000))

    def sel_rows(base, seg0):
        parts = []
        for u in range(U):
            r = _mult(base + (seg0 + u) * SEG + (SEG - PR), PR)
            parts.append(xn_scr[pl.ds(r, PR), :])
        return jnp.concatenate(parts, axis=0)

    def fill(i, lhs, prow):
        pre_scr[2 * H + i, pl.ds(prow, U * PR), :] = _dot(lhs, _w(w_ref[2 * H + fill_heads[i]]))

    def ln_sel(c, carry):
        blk = xs_ref.at[pl.ds(c * xc, xc)]
        pltpu.make_async_copy(blk, blk, sems.at[sem_xs + c]).wait()
        xv = xs_ref[pl.ds(c * xc, xc)].astype(F32).reshape(xc * PR, D)
        xp_scr[pl.ds(pl.multiple_of(c * xc * PR, xc * PR), xc * PR), :] = _ln(xv).astype(BF16)
        return carry

    with _scope('p_ln'):
        lax.fori_loop(0, NXC, ln_sel, 0)
        pin_scr[...] = jnp.zeros_like(pin_scr)
        pin2_scr[...] = jnp.zeros_like(pin2_scr)
        p_scr[0:8, :] = jnp.zeros((8, DH), F32)
        for scr in (ks_scr, vs_scr):
            scr[0:8, :] = jnp.zeros((8, DH), F32)
        wait_raw(0)
        unpack(0)

    HI = 4
    NI = H // HI
    UP = 3

    def pre_wi(slot):
        nk = H // KS
        if isinstance(slot, int):
            return slot if slot < H else (H + KS * (slot - H) if slot < H + nk else 2 * H + slot - H - nk)
        return jnp.where(slot < H, slot, jnp.where(slot < H + nk, H + KS * (slot - H), H + slot - nk))

    pre_slot = {pre_wi(t): t for t in range(2 * H)}

    def pre_iter(hd0, nh, pairs):
        for i in pairs:
            wait_raw(i)
        xp = xp_scr[0:nseg * PR, :]
        pairs = list(pairs)
        for e in range(nh):
            pre_scr[hd0 + e, 0:nseg * PR, :] = _dot(xp, _w(w_ref[pre_wi(hd0 + e)]))
            if e < nh - 1:
                take = -(-len(pairs) // (nh - 1 - e))
                for i in pairs[:take]:
                    unpack(i)
                pairs = pairs[take:]

    def pre_qk(it, carry):
        pre_iter(HI * it, HI, [UP * it + 1 + e for e in range(UP)])
        return carry

    with _scope('p_0'):
        pre_iter(0, 2, [1])
        pre_iter(2, 2, [2, 3])
    with _scope('p_qk'):
        lax.fori_loop(1, 2 * NI - 1, pre_qk, 0)
    with _scope('p_last'):
        cp_xa.wait()
        pre_iter(HI * (2 * NI - 1), HI, list(range(UP * (2 * NI - 1) + 1, 3 * HP)))
        xn_scr[0:SEG, :] = _ln(x_ref[0].astype(F32))
        lhs0 = xp_scr[0:U * PR, :]
        for i in range(NFH):
            fill(i, lhs0, 0)
    with _scope('w_wo'):
        for cp in wo_cps:
            cp.wait()
    ffn_cps = []
    for src, dst, nb in ((wg_hbm, wg_ref, NF), (wu_hbm, wu_ref, NF), (wd_hbm, wd_ref, NC)):
        for c in range(nb):
            ffn_cps.append(pltpu.make_async_copy(src.bitcast(U32).at[:, c * DH:(c + 1) * DH], dst.at[c],
                                                 sems.at[sem_ffn + len(ffn_cps)]))
            ffn_cps[-1].start()

    row = lax.broadcasted_iota(jnp.int32, (L, L), 0)
    col = lax.broadcasted_iota(jnp.int32, (L, L), 1)
    mask = (row < M) | (row >= col)
    wr = wr_ref[...].astype(F32).reshape(1, D)
    masks = {}
    for nb_ in set(nvb) - {0}:
        rr = lax.broadcasted_iota(jnp.int32, (L - 8 * nb_, L), 0)
        cc = lax.broadcasted_iota(jnp.int32, (L - 8 * nb_, L), 1)
        masks[nb_] = (rr < M) | (rr + 8 * nb_ >= cc)
    row8 = lax.broadcasted_iota(jnp.int32, (8, DH), 0)

    def vpu_offs(j):
        return list(range(0, M + 8 * j + 1)) + list(range(-1, -8, -1))

    def vpu_scores(hd, j, qb):
        b0 = koff[hd]
        qs = qb * (scale * LOG2E)
        ss = []
        for o_ in vpu_offs(j):
            sv = jnp.sum(qs * ks_scr[b0 + o_:b0 + o_ + 8, :], axis=-1, keepdims=True)
            sv = jnp.broadcast_to(sv, (8, DH))
            if o_ < 0:
                sv = jnp.where(row8 >= -o_, sv, -1e9 * LOG2E)
            ss.append(sv)
        return ss

    def vpu_pv(hd, j, ss):
        b0 = koff[hd]
        offs = vpu_offs(j)
        mx = den = acc = None
        for c0 in range(0, len(offs), CH):
            cs = ss[c0:c0 + CH]
            cm = _tree(jnp.maximum, cs if mx is None else cs + [mx])
            if mx is not None:
                alpha = jnp.exp2(mx - cm)
                den = den * alpha
                acc = acc * alpha
            mx = cm
            if SERIAL:
                for sv, o_ in zip(cs, offs[c0:c0 + CH]):
                    pv = jnp.exp2(sv - mx)
                    t = pv * vs_scr[b0 + o_:b0 + o_ + 8, :]
                    den = pv if den is None else den + pv
                    acc = t if acc is None else acc + t
            else:
                ps = [jnp.exp2(sv - mx) for sv in cs]
                ts = [pv * vs_scr[b0 + o_:b0 + o_ + 8, :] for pv, o_ in zip(ps, offs[c0:c0 + CH])]
                den = _tree(jnp.add, ps if den is None else ps + [den])
                acc = _tree(jnp.add, ts if acc is None else ts + [acc])
        return acc * pl.reciprocal(den, approx=True)

    OB = U * SEG

    def out_copy(r0, nrows, sem):
        return pltpu.make_async_copy(out_v.at[pl.ds(r0, nrows)], out_hbm.at[pl.ds(r0, nrows)], sems.at[sem])

    def layer(li):
        base = li * S
        first = li == 0
        dur_v = [32 if (hd in fill_heads or (first and 2 * H + hd in pre_slot)) else 40 for hd in range(H)]
        dur_qk = [(32 + (32 if H + hd in pre_slot else 40)) if first else 80 for hd in range(H)]
        sfx = "1" if first else "2"
        order = _step_order(H, dur_qk, dur_v, [L - 2 * sum(nvb[g * G:(g + 1) * G]) for g in range(H // G)],
                            _env("LEAD" + sfx, 32), _env("HOLD" + sfx, 9),
                            _env("FIN" + sfx, 2600 if first else 1200), _env("LMM", 155), _env("LSM", 450), _env("LPIN" + sfx, 450), _env("VD" + sfx, 0),
                            [_env("VGAP", 3) * (16 * nvb[hd] + 8 * (nvb[hd] > 1)) for hd in range(H)])


        def finish(sp, o_tok, best_v, best_s, valid):
            r0 = _mult(sp * SEG, SEG)
            xin = x_ref[sp].astype(F32) if first else xb_scr[pl.ds(r0, SEG), :]
            x1 = _rb(xin + o_tok)
            xn1 = _ln(x1)
            r = _rb(jnp.sum(xn1 * wr, axis=-1, keepdims=True))
            upd = r > best_v
            if valid is not None:
                upd = jnp.logical_and(upd, valid)
            best_v = jnp.where(upd, r, best_v)
            best_s = jnp.where(upd, sp, best_s)
            x2 = _rb(x1 + xn1)
            xa_scr[pl.ds(r0, SEG), :] = x1
            if first:
                xc_scr[pl.ds(r0, SEG), :] = xn1
                xb_scr[pl.ds(r0, SEG), :] = x2
                xn_scr[pl.ds(S + r0, SEG), :] = _ln(x2)
            else:
                xn_scr[pl.ds(r0, SEG), :] = xn1
                out_v[pl.ds(r0, SEG), :] = x2.astype(BF16)
            return best_v, best_s

        def segment(s, mem, prev_tok, best_v, best_s, valid):
            r0 = pl.multiple_of(base + s * SEG, SEG)
            p0 = pl.multiple_of(s * PR, PR)
            hh = [jnp.concatenate([mem, xn_scr[pl.ds(r0, SEG), :]], axis=0)]
            hb = [hh[0][:L0].astype(BF16)]
            q = [None] * H
            k = [None] * H
            v = [None] * H
            p = [None] * H
            il = [None] * H
            o = [None] * H
            dd = [None] * H
            pw = [None] * H
            acc = None
            nacc = 0
            za = pl.multiple_of((s >> 12) * 8, 8)
            zb = pl.multiple_of((s >> 13) * 8, 8)

            ppin = [False]

            def proj(wi, pcol):
                lhs = hh[0]
                if ppin[0]:
                    ppin[0] = False
                    z = p_scr[0:8, :]
                    top = jnp.concatenate([lhs[:8, :DH] + z, lhs[:8, DH:]], axis=1)
                    lhs = jnp.concatenate([top, lhs[8:]], axis=0)
                if pcol is None:
                    return _dot(lhs, _w(w_ref[wi]))
                lb = hb[0] if (BFL & 1) and lhs is hh[0] else lhs[:L0]
                return jnp.concatenate(
                    [_dot(lb, _w(w_ref[wi])), pre_scr[pcol, pl.ds(p0, PR), :]], axis=0)

            for kind, i in order:
                if kind == "qk":
                    q[i] = proj(i, i if first else None)
                    k[i] = proj(H + i, pre_slot.get(H + i) if first else None)
                    if nvb[i]:
                        nk = M + 8 * nvb[i]
                        ks_scr[koff[i]:koff[i] + nk, :] = k[i][:nk]
                elif kind == "s":
                    for hd in range(i * G, (i + 1) * G):
                        qm = q[hd]
                        mk = mask
                        if nvb[hd]:
                            qm = jnp.concatenate([qm[:M], qm[M + 8 * nvb[hd]:]], axis=0)
                            mk = masks[nvb[hd]]
                        if (BFL & 2) and qm.shape[0] % 16 == 0:
                            qm = qm.astype(BF16)
                        sc = _dot_nt(qm, k[hd]) * scale
                        sc = jnp.where(mk, sc, -1e9)
                        mx = jnp.max(sc, axis=-1, keepdims=True)
                        e = jnp.exp(sc - mx)
                        pn = e * pl.reciprocal(jnp.sum(e, axis=-1, keepdims=True), approx=True)
                        if (BFL & 4) and pn.shape[0] % 16 == 0:
                            pn = pn.astype(BF16)
                        p[hd] = pn
                elif kind == "ppin":
                    if PPIN and p[i * G] is not None:
                        for hd in range(i * G, (i + 1) * G):
                            p_scr[pl.ds(za + 8 + hd * L, p[hd].shape[0]), 0:L] = p[hd]
                            p[hd] = None
                        ppin[0] = True
                elif kind == "v":
                    v[i] = proj(2 * H + i, 2 * H + fill_heads.index(i) if i in fill_heads
                                else (pre_slot.get(2 * H + i) if first else None))
                    if nvb[i]:
                        nk = M + 8 * nvb[i]
                        vs_scr[koff[i]:koff[i] + nk, :] = v[i][:nk]
                elif kind == "vs":
                    hd, (sk, si) = i
                    if nvb[hd]:
                        src = {"v": v, "wo": dd, "qk": k}[sk][si]
                        pin2_scr[pl.ds(za + 8, 8), :] = src[:8, :DH]
                        z = pin2_scr[pl.ds(zb, 8), :]
                        pw[hd] = [vpu_scores(hd, j, q[hd][M + 8 * j:M + 8 * (j + 1)] + z) for j in range(nvb[hd])]
                elif kind == "pv":
                    for hd in range(i * G, (i + 1) * G):
                        if p[hd] is None:
                            p[hd] = p_scr[8 + hd * L:8 + hd * L + L - 8 * nvb[hd], 0:L]
                        om = _dot(p[hd], v[hd])
                        p[hd] = None
                        o[hd] = om
                elif kind == "wo":
                    lhs = o[i]
                    if nvb[i]:
                        if pw[i] is None:
                            pw[i] = [vpu_scores(i, j, q[i][M + 8 * j:M + 8 * (j + 1)]) for j in range(nvb[i])]
                        ov = [vpu_pv(i, j, pw[i][j]) for j in range(nvb[i])]
                        lhs = jnp.concatenate([lhs[:M]] + ov + [lhs[M:]], axis=0)
                    if i - PIN_GAP in PIN_AT:
                        z = pin_scr[pl.ds(zb, 8), 0:DH]
                        lhs = jnp.concatenate([lhs[:8] + z, lhs[8:]], axis=0)
                    dd[i] = jnp.concatenate(
                        [_dot(lhs, _w(wo_ref[c, i * (DH // 2):(i + 1) * (DH // 2), :])) for c in range(NC)],
                        axis=1)
                    if i in PIN_AT:
                        while nacc <= i - PIN_LAG:
                            acc = dd[nacc] if acc is None else acc + dd[nacc]
                            nacc += 1
                        pin_scr[pl.ds(za + 8, L), :] = acc
                elif kind == "finish":
                    sp = s - 1 if valid is None else jnp.maximum(s - 1, 0)
                    best_v, best_s = finish(sp, prev_tok, best_v, best_s, valid)
                    if first:
                        sn = jnp.minimum(s + 1, nseg - 1)
                        xn_scr[pl.ds(pl.multiple_of(sn * SEG, SEG), SEG), :] = _ln(x_ref[sn].astype(F32))
                    hh[0] = jnp.concatenate([mem, xn_scr[pl.ds(r0, SEG), :]], axis=0)
                    hb[0] = hh[0][:L0].astype(BF16)
            for j in range(nacc, H):
                acc = acc + dd[j]
            res = _rb(acc)
            return res[:M], res[M:], best_v, best_s

        def block(b, carry):
            mem, best_v, best_s = carry
            if first:
                @pl.when(b == 1)
                def _():
                    cp_xb.wait()
            else:
                @pl.when(b >= 2)
                def _():
                    out_copy(pl.multiple_of((b - 2) * OB, OB), OB, sem_o).start()
            tok = ot_scr[...]
            nb = jnp.minimum(b + 1, nblk - 1)
            for u in range(U):
                s = b * U + u
                mem, tok, best_v, best_s = segment(s, mem, tok, best_v, best_s, (s > 0) if u == 0 else None)
                if u < U - 1:
                    if first:
                        lhs = xp_scr[pl.ds(pl.multiple_of(nb * U * PR, U * PR), U * PR), :]
                    else:
                        lhs = sel_rows(base, nb * U).astype(BF16)
                    for i in range(u * NFILL, (u + 1) * NFILL):
                        fill(i, lhs, pl.multiple_of((b + 1) * U * PR, U * PR))
            ot_scr[...] = tok
            return mem, best_v, best_s

        ot_scr[...] = jnp.zeros_like(ot_scr)
        init = (mem0_ref[...].astype(F32),
                jnp.full((SEG, 1), -jnp.inf, F32),
                jnp.zeros((SEG, 1), jnp.int32))
        with _scope('main%d' % li):
            _, best_v, best_s = lax.fori_loop(0, nblk, block, init)
        best_v, best_s = finish(nseg - 1, ot_scr[...], best_v, best_s, None)
        if first:
            for cp in ffn_cps:
                cp.wait()
        else:
            out_copy((nblk - 2) * OB, 2 * OB, sem_o).start()

        vmax = jnp.max(best_v, axis=0, keepdims=True)
        tok = best_s * SEG + lax.broadcasted_iota(jnp.int32, (SEG, 1), 0)
        idx = jnp.min(jnp.where(best_v == vmax, tok, S))
        idx = jnp.clip(idx, 0, S - 1)
        xs = xc_scr[pl.ds(idx, 1), :] if first else xn_scr[pl.ds(idx, 1), :]
        x1 = xa_scr[pl.ds(idx, 1), :]
        xs8 = jnp.broadcast_to(xs, (8, D))
        g = _rb(jnp.concatenate([_dot(xs8, _w(wg_ref[c])) for c in range(NF)], axis=1))
        u = _rb(jnp.concatenate([_dot(xs8, _w(wu_ref[c])) for c in range(NF)], axis=1))
        g = _rb(g * _rb(jax.nn.sigmoid(g)))
        gu = _rb(g * u)
        y = _rb(jnp.concatenate([_dot(gu, _w(wd_ref[c])) for c in range(NC)], axis=1))
        y = _rb(y * _rb(jax.nn.sigmoid(vmax)))
        new = _rb(x1 + _rb(xs + y[0:1]))
        return idx, new

    idx, new = layer(0)
    xb_scr[pl.ds(idx, 1), :] = new
    xn_scr[pl.ds(S + idx, 1), :] = _ln(new)
    lhs0 = sel_rows(S, 0)
    for i in range(NFH):
        fill(i, lhs0, 0)

    idx, new = layer(1)
    out_copy(0, S, sem_o).wait()
    b0 = pl.multiple_of((idx // 16) * 16, 16)
    blk = out_v[pl.ds(b0, 16), :].astype(F32)
    rid = b0 + lax.broadcasted_iota(jnp.int32, (16, D), 0)
    out_v[pl.ds(b0, 16), :] = jnp.where(rid == idx, new, blk).astype(BF16)
    cp = out_copy(b0, 16, sem_o2)
    cp.start()
    cp.wait()


@jax.jit
def pallas_interleave_layers__memory_aug_recurrent_mem_tr__moe_arch_mod__prompt_kernel(
    A_x, A_mem0, A_Wq, A_Wk, A_Wv, A_Wo, A_seg_len, B_x, B_w_r, B_w_gate, B_w_up, B_w_down,
):
    B, S, D = A_x.shape
    _, H, DH = A_Wq.shape
    M = A_mem0.shape[1]
    F = B_w_gate.shape[1]
    assert B == 1 and S % (SEG * U) == 0
    nseg = S // SEG
    kern = functools.partial(_kernel, S=S, D=D, H=H, DH=DH, M=M, F=F)
    hbm = pl.BlockSpec(memory_space=pl.ANY)
    vm = pl.BlockSpec(memory_space=pltpu.VMEM)
    nsem = 8 + 3 * (H // 2) + D // DH + 2 * (F // DH) + D // DH
    out = pl.pallas_call(
        kern,
        out_shape=jax.ShapeDtypeStruct((S, D), BF16),
        in_specs=[hbm, vm, hbm, hbm, hbm, hbm, vm, hbm, hbm, hbm],
        out_specs=hbm,
        scratch_shapes=[
            pltpu.VMEM((nseg, SEG, D), BF16),
            pltpu.VMEM((nseg, PR, D), BF16),
            pltpu.VMEM((nseg * PR, D), BF16),
            pltpu.VMEM((3 * (H // 2), D, DH), U32),
            pltpu.VMEM((3 * H, D // 2, DH), U32),
            pltpu.VMEM((D // DH, H * DH // 2, DH), U32),
            pltpu.VMEM((F // DH, D // 2, DH), U32), pltpu.VMEM((F // DH, D // 2, DH), U32),
            pltpu.VMEM((D // DH, F // 2, DH), U32),
            pltpu.VMEM((2 * H + NFILL * (U - 1), (nseg + U) * PR, DH), F32),
            pltpu.VMEM((2 * S, D), F32),
            pltpu.VMEM((S, D), F32), pltpu.VMEM((S, D), F32), pltpu.VMEM((S, D), F32),
            pltpu.VMEM((SEG, D), F32),
            pltpu.VMEM((M + SEG + 8, D), F32),
            pltpu.VMEM((S, D), BF16),
            pltpu.VMEM((8 + H * (M + 16), DH), F32), pltpu.VMEM((8 + H * (M + 16), DH), F32),
            pltpu.VMEM((16, DH), F32),
            pltpu.VMEM((8 + H * (M + SEG), DH), F32),
            pltpu.SemaphoreType.DMA((nsem,))],
        compiler_params=pltpu.CompilerParams(vmem_limit_bytes=110 * 1024 * 1024),
    )(A_x.reshape(nseg, SEG, D), A_mem0.reshape(M, D), A_Wq, A_Wk, A_Wv,
      A_Wo.reshape(H * DH, D), B_w_r, B_w_gate, B_w_up, B_w_down)
    return out.reshape(B, S, D)
```

```python
import functools
import numpy as np
import jax
import jax.numpy as jnp
from jax import lax
import jax.experimental.pallas as pl
import jax.experimental.pallas.tpu as pltpu

F32 = jnp.float32
BF16 = jnp.bfloat16
U32 = jnp.uint32
SEG = 32
EPS = 1e-05
G = 4
PR = 8


def _env(name, default):
    return default


U = _env("U", 4)
NFILL = _env("NFILL", 5)
PIN_LAG = _env("PIN_LAG", 4)
PIN_GAP = _env("PIN_GAP", 2)
PIN_AT = [int(t) for t in "4,6,8,10,12,14,16,18,20,22,24,26,28,29".split(",")]
NVB = _env("NVB", 1)
VB2 = [int(t) for t in "".split(",") if t]
PPIN = _env("PPIN", 0) == 1
KS = _env("KS", 1)
BFL = _env("BFL", 5)
CH = _env("CH", 8)
SERIAL = _env("SERIAL", 1)
FFN_EARLY = _env("FFN_EARLY", 1)
LOG2E = 1.4426950408889634
SCOPES = _env("SCOPES", 0)


class _NoScope:
    def __enter__(self):
        return self

    def __exit__(self, *a):
        return False


def _scope(name):
    return jax.named_scope(name) if SCOPES else _NoScope()


def _rb(x):
    return x.astype(BF16).astype(F32)


def _ln(x):
    d = x.shape[-1]
    mu = jnp.sum(x, axis=-1, keepdims=True) * (1.0 / d)
    c = x - mu
    var = jnp.sum(c * c, axis=-1, keepdims=True) * (1.0 / d)
    m = _rb(mu)
    v = _rb(var)
    den = _rb(jnp.sqrt(_rb(v + EPS)))
    return _rb(_rb(x - m) / den)


def _w(x):
    return pltpu.bitcast(x, BF16)


def _dot(a, b):
    return lax.dot_general(a, b, (((1,), (0,)), ((), ())), preferred_element_type=F32)


def _dot_nt(a, b):
    return lax.dot_general(a, b, (((1,), (1,)), ((), ())), preferred_element_type=F32)


def _tree(f, xs):
    xs = list(xs)
    while len(xs) > 1:
        xs = [f(xs[i], xs[i + 1]) if i + 1 < len(xs) else xs[i] for i in range(0, len(xs), 2)]
    return xs[0]


def _mult(r, m):
    return r if isinstance(r, int) else pl.multiple_of(r, m)


def _step_order(H, dur_qk, dur_v, dur_a, lead, hold, fin_at, l_mm, l_sm, l_pin, vd, vgap):
    NG = H // G
    out = []
    t = 0
    nqk = nv = nwo = ns = npv = 0
    qk_end = [0] * H
    v_end = [0] * H
    s_end = [0] * NG
    pv_end = [0] * NG
    last = None
    fin_done = False
    npin = 0
    ends = {}
    while nwo < H:
        if not fin_done and t >= fin_at:
            out.append(("finish", 0))
            fin_done = True
        s_ok = ns < NG and nqk >= (ns + 1) * G and t >= qk_end[(ns + 1) * G - 1] + l_mm
        pv_ok = (npv < ns and nv >= (npv + 1) * G and t >= v_end[(npv + 1) * G - 1] + l_mm
                 and t >= s_end[npv] + l_sm)
        qk_ok = nqk < H
        v_ok = nv < H and (nqk >= H or nv + lead < nqk)
        wo_ok = (nwo < npv * G and t >= pv_end[nwo // G] + l_mm and (nv >= H or nwo + hold < nv))
        if s_ok:
            out.append(("s", ns)); t += dur_a[ns]; s_end[ns] = t; ns += 1
        elif pv_ok:
            out.append(("pv", npv)); t += dur_a[npv]; pv_end[npv] = t; npv += 1
        else:
            cand = [c for c, ok in (("qk", qk_ok), ("v", v_ok), ("wo", wo_ok)) if ok]
            if not cand:
                t += 4
                continue
            rot = {"qk": ("v", "wo", "qk"), "v": ("wo", "qk", "v"), "wo": ("qk", "v", "wo"),
                   None: ("qk", "v", "wo")}[last]
            c = [x for x in rot if x in cand][0]
            last = c
            if c in ("qk", "v") and npin < ns and t >= s_end[npin] + l_pin:
                while npin < ns and t >= s_end[npin] + l_pin:
                    out.append(("ppin", npin))
                    npin += 1
            if c == "qk":
                out.append(("qk", nqk)); t += dur_qk[nqk]; qk_end[nqk] = t; ends[("qk", nqk)] = t; nqk += 1
            elif c == "v":
                out.append(("v", nv)); t += dur_v[nv]; v_end[nv] = t; ends[("v", nv)] = t; nv += 1
            else:
                out.append(("wo", nwo)); t += 40; ends[("wo", nwo)] = t; nwo += 1
    if vd:
        tp = [0] * H
        for hd in range(H - 1, -1, -1):
            tp[hd] = ends[("wo", hd)] - 40 - vd
            if hd + 1 < H:
                tp[hd] = min(tp[hd], tp[hd + 1] - vgap[hd])
        after = {}
        for hd in range(H):
            cands = [key for key, e in ends.items() if e + 140 <= tp[hd] and e >= ends[("qk", hd)]]
            if cands:
                src = max(cands, key=lambda key: ends[key])
                after.setdefault(src, []).append(hd)
        out2 = []
        for op in out:
            out2.append(op)
            for hd in after.get(op, []):
                out2.append(("vs", (hd, op)))
        out = out2
    return out


def _kernel(x_hbm, mem0_ref, wq_hbm, wk_hbm, wv_hbm, wo_hbm, wr_ref, wg_hbm, wu_hbm, wd_hbm,
            out_hbm,
            x_ref, xs_ref, xp_scr, raw_scr, w_ref, wo_ref, wg_ref, wu_ref, wd_ref,
            pre_scr, xn_scr, xa_scr, xc_scr, xb_scr, ot_scr, pin_scr, out_v, ks_scr, vs_scr, pin2_scr, p_scr, zero_smem, sems,
            *, S, D, H, DH, M, F):
    L = M + SEG
    L0 = L - PR
    nseg = S // SEG
    nblk = nseg // U
    HP = H // 2
    NC = D // DH
    NF = F // DH
    NFH = NFILL * (U - 1)
    fill_heads = list(range(H - NFH, H))
    scale = float(np.asarray(DH ** -0.5).astype(BF16))
    nvb = [NVB + (1 if hd in VB2 else 0) for hd in range(H)]
    koff = [8 + sum(M + 8 * n for n in nvb[:hd]) for hd in range(H)]

    NXC = 4
    xc = nseg // NXC
    HI = 4
    UP = 3
    NA = _env("NA", 3)
    NPRE = 2 * H
    NB = (NPRE - HI * (NA + 1)) // (2 * HI) - 1
    hb0 = HI * (NA + 1)
    pb0 = UP * (NA + 1)
    groups = [(0, 1), (1, 1), (2, 2), (4, 2)] + [(UP * it, UP) for it in range(2, NA + 1)]
    groups += [(pb0 + 2 * UP * it, 2 * UP) for it in range(NB)]
    groups += [(pb0 + 2 * UP * NB, 3 * HP - pb0 - 2 * UP * NB)]
    sem_xs, sem_x, sem_o, sem_o2, sem_xb, sem_wo, sem_ffn = 0, NXC, NXC + 1, NXC + 2, NXC + 3, NXC + 4, NXC + 5
    sem_w = NXC + 6

    for c in range(NXC):
        pltpu.make_async_copy(x_hbm.at[c * xc:(c + 1) * xc, SEG - PR:SEG, :],
                              xs_ref.at[c * xc:(c + 1) * xc], sems.at[sem_xs + c]).start()
    XA = U + 1
    cp_xa = pltpu.make_async_copy(x_hbm.at[0:XA], x_ref.at[0:XA], sems.at[sem_x])
    cp_xb = pltpu.make_async_copy(x_hbm.at[XA:nseg], x_ref.at[XA:nseg], sems.at[sem_xb])
    X_AFTER = _env("X_AFTER", 30)
    w32 = [w.bitcast(U32) for w in (wq_hbm, wk_hbm, wv_hbm)]
    for gi, (g0, gn) in enumerate(groups):
        for i in range(g0, g0 + gn):
            pltpu.make_async_copy(w32[i // HP].at[:, i % HP, :], raw_scr.at[i], sems.at[sem_w + gi]).start()
            if i == X_AFTER:
                cp_xa.start()
    cp_wo = pltpu.make_async_copy(wo_hbm.bitcast(U32), wo_ref, sems.at[sem_wo])
    cp_wo.start()
    cp_xb.start()
    ffn_cps = [pltpu.make_async_copy(src.bitcast(U32), dst, sems.at[sem_ffn])
               for src, dst in ((wg_hbm, wg_ref), (wu_hbm, wu_ref), (wd_hbm, wd_ref))]
    if FFN_EARLY:
        for cp in ffn_cps:
            cp.start()
    zero_smem[0] = 0

    def wait_group(gi, g0, gn):
        blk = raw_scr.at[pl.ds(g0, gn)]
        pltpu.make_async_copy(blk, blk, sems.at[sem_w + gi]).wait()

    def unpack(i):
        for cb in range(D // 128):
            a = raw_scr[i, pl.ds(cb * 128, 64, stride=2), :]
            b = raw_scr[i, pl.ds(cb * 128 + 1, 64, stride=2), :]
            w_ref[2 * i, cb * 64:(cb + 1) * 64, :] = (a & jnp.uint32(0xFFFF)) | (b << 16)
            w_ref[2 * i + 1, cb * 64:(cb + 1) * 64, :] = (a >> 16) | (b & jnp.uint32(0xFFFF0000))

    def sel_rows(base, seg0):
        parts = []
        for u in range(U):
            r = _mult(base + (seg0 + u) * SEG + (SEG - PR), PR)
            parts.append(xn_scr[pl.ds(r, PR), :])
        return jnp.concatenate(parts, axis=0)

    def fill(i, lhs, prow):
        pre_scr[2 * H + i, pl.ds(prow, U * PR), :] = _dot(lhs, _w(w_ref[2 * H + fill_heads[i]]))

    def ln_sel(c, carry):
        blk = xs_ref.at[pl.ds(c * xc, xc)]
        pltpu.make_async_copy(blk, blk, sems.at[sem_xs + c]).wait()
        xv = xs_ref[pl.ds(c * xc, xc)].astype(F32).reshape(xc * PR, D)
        xp_scr[pl.ds(pl.multiple_of(c * xc * PR, xc * PR), xc * PR), :] = _ln(xv).astype(BF16)
        return carry

    with _scope('p_ln'):
        lax.fori_loop(0, NXC, ln_sel, 0)
        pin_scr[...] = jnp.zeros_like(pin_scr)
        pin2_scr[...] = jnp.zeros_like(pin2_scr)
        p_scr[0:8, :] = jnp.zeros((8, DH), F32)
        for scr in (ks_scr, vs_scr):
            scr[0:8, :] = jnp.zeros((8, DH), F32)
        wait_group(0, *groups[0])
        unpack(0)

    def pre_wi(slot):
        nk = H // KS
        if isinstance(slot, int):
            return slot if slot < H else (H + KS * (slot - H) if slot < H + nk else 2 * H + slot - H - nk)
        return jnp.where(slot < H, slot, jnp.where(slot < H + nk, H + KS * (slot - H), H + slot - nk))

    pre_slot = {pre_wi(t): t for t in range(NPRE)}

    def pre_iter(hd0, nh, gi, g0, gn):
        wait_group(gi, g0, gn)
        xp = xp_scr[0:nseg * PR, :]
        pairs = [g0 + e for e in range(gn)]
        for e in range(nh):
            pre_scr[hd0 + e, 0:nseg * PR, :] = _dot(xp, _w(w_ref[pre_wi(hd0 + e)]))
            if e >= 1:
                take = -(-len(pairs) // (nh - e))
                for i in pairs[:take]:
                    unpack(i)
                pairs = pairs[take:]

    def pre_a(it, carry):
        pre_iter(HI * it, HI, 2 + it, UP * it, UP)
        return carry

    def pre_b(it, carry):
        pre_iter(hb0 + 2 * HI * it, 2 * HI, 3 + NA + it, pb0 + 2 * UP * it, 2 * UP)
        return carry

    dz = zero_smem[0]
    with _scope('p_0'):
        pre_iter(0, 2, 1, *groups[1])
        pre_iter(2, 2, 2, *groups[2])
        pre_iter(HI, HI, 3, groups[3][0] + dz, groups[3][1])
    with _scope('p_a'):
        lax.fori_loop(2, NA + 1, pre_a, 0)
    with _scope('p_b'):
        lax.fori_loop(0, NB, pre_b, 0)
    with _scope('p_last'):
        cp_xa.wait()
        pre_iter(hb0 + 2 * HI * NB, 2 * HI, len(groups) - 1, groups[-1][0] + dz, groups[-1][1])
        xn_scr[0:SEG, :] = _ln(x_ref[0].astype(F32))
        lhs0 = xp_scr[0:U * PR, :]
        for i in range(NFH):
            fill(i, lhs0, 0)
    with _scope('w_wo'):
        cp_wo.wait()
    if not FFN_EARLY:
        for cp in ffn_cps:
            cp.start()

    row = lax.broadcasted_iota(jnp.int32, (L, L), 0)
    col = lax.broadcasted_iota(jnp.int32, (L, L), 1)
    mask = (row < M) | (row >= col)
    wr = wr_ref[...].astype(F32).reshape(1, D)
    masks = {}
    for nb_ in set(nvb) - {0}:
        rr = lax.broadcasted_iota(jnp.int32, (L - 8 * nb_, L), 0)
        cc = lax.broadcasted_iota(jnp.int32, (L - 8 * nb_, L), 1)
        masks[nb_] = (rr < M) | (rr + 8 * nb_ >= cc)
    row8 = lax.broadcasted_iota(jnp.int32, (8, DH), 0)

    def vpu_offs(j):
        return list(range(0, M + 8 * j + 1)) + list(range(-1, -8, -1))

    def vpu_scores(hd, j, qb):
        b0 = koff[hd]
        qs = qb * (scale * LOG2E)
        ss = []
        for o_ in vpu_offs(j):
            sv = jnp.sum(qs * ks_scr[b0 + o_:b0 + o_ + 8, :], axis=-1, keepdims=True)
            sv = jnp.broadcast_to(sv, (8, DH))
            if o_ < 0:
                sv = jnp.where(row8 >= -o_, sv, -1e9 * LOG2E)
            ss.append(sv)
        return ss

    def vpu_pv(hd, j, ss):
        b0 = koff[hd]
        offs = vpu_offs(j)
        mx = den = acc = None
        for c0 in range(0, len(offs), CH):
            cs = ss[c0:c0 + CH]
            cm = _tree(jnp.maximum, cs if mx is None else cs + [mx])
            if mx is not None:
                alpha = jnp.exp2(mx - cm)
                den = den * alpha
                acc = acc * alpha
            mx = cm
            if SERIAL:
                for sv, o_ in zip(cs, offs[c0:c0 + CH]):
                    pv = jnp.exp2(sv - mx)
                    t = pv * vs_scr[b0 + o_:b0 + o_ + 8, :]
                    den = pv if den is None else den + pv
                    acc = t if acc is None else acc + t
            else:
                ps = [jnp.exp2(sv - mx) for sv in cs]
                ts = [pv * vs_scr[b0 + o_:b0 + o_ + 8, :] for pv, o_ in zip(ps, offs[c0:c0 + CH])]
                den = _tree(jnp.add, ps if den is None else ps + [den])
                acc = _tree(jnp.add, ts if acc is None else ts + [acc])
        return acc * pl.reciprocal(den, approx=True)

    OB = U * SEG

    def out_copy(r0, nrows, sem):
        return pltpu.make_async_copy(out_v.at[pl.ds(r0, nrows)], out_hbm.at[pl.ds(r0, nrows)], sems.at[sem])

    def layer(li):
        base = li * S
        first = li == 0
        dur_v = [32 if (hd in fill_heads or (first and 2 * H + hd in pre_slot)) else 40 for hd in range(H)]
        dur_qk = [(32 + (32 if H + hd in pre_slot else 40)) if first else 80 for hd in range(H)]
        sfx = "1" if first else "2"
        order = _step_order(H, dur_qk, dur_v, [L - 2 * sum(nvb[g * G:(g + 1) * G]) for g in range(H // G)],
                            _env("LEAD" + sfx, 32), _env("HOLD" + sfx, 9),
                            _env("FIN" + sfx, 2600 if first else 1200), _env("LMM", 155), _env("LSM", 450), _env("LPIN" + sfx, 450), _env("VD" + sfx, 0),
                            [_env("VGAP", 3) * (16 * nvb[hd] + 8 * (nvb[hd] > 1)) for hd in range(H)])


        def finish(sp, o_tok, best_v, best_s, valid):
            r0 = _mult(sp * SEG, SEG)
            xin = x_ref[sp].astype(F32) if first else xb_scr[pl.ds(r0, SEG), :]
            x1 = _rb(xin + o_tok)
            xn1 = _ln(x1)
            r = _rb(jnp.sum(xn1 * wr, axis=-1, keepdims=True))
            upd = r > best_v
            if valid is not None:
                upd = jnp.logical_and(upd, valid)
            best_v = jnp.where(upd, r, best_v)
            best_s = jnp.where(upd, sp, best_s)
            x2 = _rb(x1 + xn1)
            xa_scr[pl.ds(r0, SEG), :] = x1
            if first:
                xc_scr[pl.ds(r0, SEG), :] = xn1
                xb_scr[pl.ds(r0, SEG), :] = x2
                xn_scr[pl.ds(S + r0, SEG), :] = _ln(x2)
            else:
                xn_scr[pl.ds(r0, SEG), :] = xn1
                out_v[pl.ds(r0, SEG), :] = x2.astype(BF16)
            return best_v, best_s

        def segment(s, mem, prev_tok, best_v, best_s, valid):
            r0 = pl.multiple_of(base + s * SEG, SEG)
            p0 = pl.multiple_of(s * PR, PR)
            hh = [jnp.concatenate([mem, xn_scr[pl.ds(r0, SEG), :]], axis=0)]
            hb = [hh[0][:L0].astype(BF16)]
            q = [None] * H
            k = [None] * H
            v = [None] * H
            p = [None] * H
            il = [None] * H
            o = [None] * H
            dd = [None] * H
            pw = [None] * H
            acc = None
            nacc = 0
            za = pl.multiple_of((s >> 12) * 8, 8)
            zb = pl.multiple_of((s >> 13) * 8, 8)

            ppin = [False]

            def proj(wi, pcol):
                lhs = hh[0]
                if ppin[0]:
                    ppin[0] = False
                    z = p_scr[0:8, :]
                    top = jnp.concatenate([lhs[:8, :DH] + z, lhs[:8, DH:]], axis=1)
                    lhs = jnp.concatenate([top, lhs[8:]], axis=0)
                if pcol is None:
                    return _dot(lhs, _w(w_ref[wi]))
                lb = hb[0] if (BFL & 1) and lhs is hh[0] else lhs[:L0]
                return jnp.concatenate(
                    [_dot(lb, _w(w_ref[wi])), pre_scr[pcol, pl.ds(p0, PR), :]], axis=0)

            for kind, i in order:
                if kind == "qk":
                    q[i] = proj(i, i if first else None)
                    k[i] = proj(H + i, pre_slot.get(H + i) if first else None)
                    if nvb[i]:
                        nk = M + 8 * nvb[i]
                        ks_scr[koff[i]:koff[i] + nk, :] = k[i][:nk]
                elif kind == "s":
                    for hd in range(i * G, (i + 1) * G):
                        qm = q[hd]
                        mk = mask
                        if nvb[hd]:
                            qm = jnp.concatenate([qm[:M], qm[M + 8 * nvb[hd]:]], axis=0)
                            mk = masks[nvb[hd]]
                        if (BFL & 2) and qm.shape[0] % 16 == 0:
                            qm = qm.astype(BF16)
                        sc = _dot_nt(qm, k[hd]) * (scale * LOG2E)
                        sc = jnp.where(mk, sc, -1e9 * LOG2E)
                        mx = jnp.max(sc, axis=-1, keepdims=True)
                        e = jnp.exp2(sc - mx)
                        pn = e * pl.reciprocal(jnp.sum(e, axis=-1, keepdims=True), approx=True)
                        if (BFL & 4) and pn.shape[0] % 16 == 0:
                            pn = pn.astype(BF16)
                        p[hd] = pn
                elif kind == "ppin":
                    if PPIN and p[i * G] is not None:
                        for hd in range(i * G, (i + 1) * G):
                            p_scr[pl.ds(za + 8 + hd * L, p[hd].shape[0]), 0:L] = p[hd]
                            p[hd] = None
                        ppin[0] = True
                elif kind == "v":
                    v[i] = proj(2 * H + i, 2 * H + fill_heads.index(i) if i in fill_heads
                                else (pre_slot.get(2 * H + i) if first else None))
                    if nvb[i]:
                        nk = M + 8 * nvb[i]
                        vs_scr[koff[i]:koff[i] + nk, :] = v[i][:nk]
                elif kind == "vs":
                    hd, (sk, si) = i
                    if nvb[hd]:
                        src = {"v": v, "wo": dd, "qk": k}[sk][si]
                        pin2_scr[pl.ds(za + 8, 8), :] = src[:8, :DH]
                        z = pin2_scr[pl.ds(zb, 8), :]
                        pw[hd] = [vpu_scores(hd, j, q[hd][M + 8 * j:M + 8 * (j + 1)] + z) for j in range(nvb[hd])]
                elif kind == "pv":
                    for hd in range(i * G, (i + 1) * G):
                        if p[hd] is None:
                            p[hd] = p_scr[8 + hd * L:8 + hd * L + L - 8 * nvb[hd], 0:L]
                        om = _dot(p[hd], v[hd])
                        p[hd] = None
                        o[hd] = om
                elif kind == "wo":
                    lhs = o[i]
                    if nvb[i]:
                        if pw[i] is None:
                            pw[i] = [vpu_scores(i, j, q[i][M + 8 * j:M + 8 * (j + 1)]) for j in range(nvb[i])]
                        ov = [vpu_pv(i, j, pw[i][j]) for j in range(nvb[i])]
                        lhs = jnp.concatenate([lhs[:M]] + ov + [lhs[M:]], axis=0)
                    if i - PIN_GAP in PIN_AT:
                        z = pin_scr[pl.ds(zb, 8), 0:DH]
                        lhs = jnp.concatenate([lhs[:8] + z, lhs[8:]], axis=0)
                    dd[i] = jnp.concatenate(
                        [_dot(lhs, _w(wo_ref[i * (DH // 2):(i + 1) * (DH // 2), c * DH:(c + 1) * DH])) for c in range(NC)],
                        axis=1)
                    if i in PIN_AT:
                        while nacc <= i - PIN_LAG:
                            acc = dd[nacc] if acc is None else acc + dd[nacc]
                            nacc += 1
                        pin_scr[pl.ds(za + 8, L), :] = acc
                elif kind == "finish":
                    sp = s - 1 if valid is None else jnp.maximum(s - 1, 0)
                    best_v, best_s = finish(sp, prev_tok, best_v, best_s, valid)
                    if first:
                        sn = jnp.minimum(s + 1, nseg - 1)
                        xn_scr[pl.ds(pl.multiple_of(sn * SEG, SEG), SEG), :] = _ln(x_ref[sn].astype(F32))
                    hh[0] = jnp.concatenate([mem, xn_scr[pl.ds(r0, SEG), :]], axis=0)
                    hb[0] = hh[0][:L0].astype(BF16)
            for j in range(nacc, H):
                acc = acc + dd[j]
            res = _rb(acc)
            return res[:M], res[M:], best_v, best_s

        def block(b, carry):
            mem, best_v, best_s = carry
            if first:
                @pl.when(b == 1)
                def _():
                    cp_xb.wait()
            else:
                @pl.when(b >= 2)
                def _():
                    out_copy(pl.multiple_of((b - 2) * OB, OB), OB, sem_o).start()
            tok = ot_scr[...]
            nb = jnp.minimum(b + 1, nblk - 1)
            for u in range(U):
                s = b * U + u
                mem, tok, best_v, best_s = segment(s, mem, tok, best_v, best_s, (s > 0) if u == 0 else None)
                if u < U - 1:
                    prow = (b + 1) * U * PR
                    if first:
                        lhs = jnp.where(b == nblk - 1, sel_rows(S, 0).astype(BF16),
                                        xp_scr[pl.ds(pl.multiple_of(nb * U * PR, U * PR), U * PR), :])
                        prow = jnp.where(b == nblk - 1, 0, prow)
                    else:
                        lhs = sel_rows(base, nb * U).astype(BF16)
                    for i in range(u * NFILL, (u + 1) * NFILL):
                        fill(i, lhs, pl.multiple_of(prow, U * PR))
            ot_scr[...] = tok
            return mem, best_v, best_s

        ot_scr[...] = jnp.zeros_like(ot_scr)
        init = (mem0_ref[...].astype(F32),
                jnp.full((SEG, 1), -jnp.inf, F32),
                jnp.zeros((SEG, 1), jnp.int32))
        with _scope('main%d' % li):
            _, best_v, best_s = lax.fori_loop(0, nblk, block, init)
        if first:
            for cp in ffn_cps:
                cp.wait()
        best_v, best_s = finish(nseg - 1, ot_scr[...], best_v, best_s, None)
        if not first:
            out_copy((nblk - 2) * OB, 2 * OB, sem_o).start()

        vmax = jnp.max(best_v, axis=0, keepdims=True)
        tok = best_s * SEG + lax.broadcasted_iota(jnp.int32, (SEG, 1), 0)
        idx = jnp.min(jnp.where(best_v == vmax, tok, S))
        idx = jnp.clip(idx, 0, S - 1)
        xs = xc_scr[pl.ds(idx, 1), :] if first else xn_scr[pl.ds(idx, 1), :]
        x1 = xa_scr[pl.ds(idx, 1), :]
        xs8 = jnp.broadcast_to(xs, (8, D))
        g = _rb(_dot(xs8, _w(wg_ref[...])))
        u = _rb(_dot(xs8, _w(wu_ref[...])))
        g = _rb(g * _rb(jax.nn.sigmoid(g)))
        gu = _rb(g * u)
        y = _rb(_dot(gu, _w(wd_ref[...])))
        y = _rb(y * _rb(jax.nn.sigmoid(vmax)))
        new = _rb(x1 + _rb(xs + y[0:1]))
        return idx, new

    idx, new = layer(0)
    xb_scr[pl.ds(idx, 1), :] = new
    xn_scr[pl.ds(S + idx, 1), :] = _ln(new)

    @pl.when(idx < U * SEG)
    def _():
        lhs0 = sel_rows(S, 0)
        for i in range(NFH):
            fill(i, lhs0, 0)

    idx, new = layer(1)
    out_copy(0, S, sem_o).wait()
    b0 = pl.multiple_of((idx // 16) * 16, 16)
    blk = out_v[pl.ds(b0, 16), :].astype(F32)
    rid = b0 + lax.broadcasted_iota(jnp.int32, (16, D), 0)
    out_v[pl.ds(b0, 16), :] = jnp.where(rid == idx, new, blk).astype(BF16)
    cp = out_copy(b0, 16, sem_o2)
    cp.start()
    cp.wait()


@jax.jit
def pallas_interleave_layers__memory_aug_recurrent_mem_tr__moe_arch_mod__prompt_kernel(
    A_x, A_mem0, A_Wq, A_Wk, A_Wv, A_Wo, A_seg_len, B_x, B_w_r, B_w_gate, B_w_up, B_w_down,
):
    B, S, D = A_x.shape
    _, H, DH = A_Wq.shape
    M = A_mem0.shape[1]
    F = B_w_gate.shape[1]
    assert B == 1 and S % (SEG * U) == 0
    nseg = S // SEG
    kern = functools.partial(_kernel, S=S, D=D, H=H, DH=DH, M=M, F=F)
    hbm = pl.BlockSpec(memory_space=pl.ANY)
    vm = pl.BlockSpec(memory_space=pltpu.VMEM)
    nsem = 22
    out = pl.pallas_call(
        kern,
        out_shape=jax.ShapeDtypeStruct((S, D), BF16),
        in_specs=[hbm, vm, hbm, hbm, hbm, hbm, vm, hbm, hbm, hbm],
        out_specs=hbm,
        scratch_shapes=[
            pltpu.VMEM((nseg, SEG, D), BF16),
            pltpu.VMEM((nseg, PR, D), BF16),
            pltpu.VMEM((nseg * PR, D), BF16),
            pltpu.VMEM((3 * (H // 2), D, DH), U32),
            pltpu.VMEM((3 * H, D // 2, DH), U32),
            pltpu.VMEM((H * DH // 2, D), U32),
            pltpu.VMEM((D // 2, F), U32), pltpu.VMEM((D // 2, F), U32),
            pltpu.VMEM((F // 2, D), U32),
            pltpu.VMEM((2 * H + NFILL * (U - 1), (nseg + U) * PR, DH), F32),
            pltpu.VMEM((2 * S, D), F32),
            pltpu.VMEM((S, D), F32), pltpu.VMEM((S, D), F32), pltpu.VMEM((S, D), F32),
            pltpu.VMEM((SEG, D), F32),
            pltpu.VMEM((M + SEG + 8, D), F32),
            pltpu.VMEM((S, D), BF16),
            pltpu.VMEM((8 + H * (M + 16), DH), F32), pltpu.VMEM((8 + H * (M + 16), DH), F32),
            pltpu.VMEM((16, DH), F32),
            pltpu.VMEM((8 + H * (M + SEG), DH), F32),
            pltpu.SMEM((1,), jnp.int32),
            pltpu.SemaphoreType.DMA((nsem,))],
        compiler_params=pltpu.CompilerParams(vmem_limit_bytes=110 * 1024 * 1024),
    )(A_x.reshape(nseg, SEG, D), A_mem0.reshape(M, D), A_Wq, A_Wk, A_Wv,
      A_Wo.reshape(H * DH, D), B_w_r, B_w_gate, B_w_up, B_w_down)
    return out.reshape(B, S, D)
```

```python
import functools
import numpy as np
import jax
import jax.numpy as jnp
from jax import lax
import jax.experimental.pallas as pl
import jax.experimental.pallas.tpu as pltpu

F32 = jnp.float32
BF16 = jnp.bfloat16
U32 = jnp.uint32
SEG = 32
EPS = 1e-05
G = 4
PR = 8


def _env(name, default):
    return default


US = (_env("U1", 4), _env("U2", 4))
NFILLS = (_env("NFILL1", 4), _env("NFILL2", 4))
NVB = _env("NVB", 1)
VB2 = [int(t) for t in "".split(",") if t]
PPIN = _env("PPIN", 0) == 1
KS = _env("KS", 1)
BFL = _env("BFL", 5)
SERIAL = _env("SERIAL", 1)
FFN_EARLY = _env("FFN_EARLY", 1)
LOG2E = 1.4426950408889634
SCOPES = _env("SCOPES", 0)


class _NoScope:
    def __enter__(self):
        return self

    def __exit__(self, *a):
        return False


def _scope(name):
    return jax.named_scope(name) if SCOPES else _NoScope()


def _rb(x):
    return x.astype(BF16).astype(F32)


def _ln(x):
    d = x.shape[-1]
    mu = jnp.sum(x, axis=-1, keepdims=True) * (1.0 / d)
    c = x - mu
    var = jnp.sum(c * c, axis=-1, keepdims=True) * (1.0 / d)
    m = _rb(mu)
    v = _rb(var)
    den = _rb(jnp.sqrt(_rb(v + EPS)))
    return _rb(_rb(x - m) / den)


def _w(x):
    return pltpu.bitcast(x, BF16)


def _dot(a, b):
    return lax.dot_general(a, b, (((1,), (0,)), ((), ())), preferred_element_type=F32)


def _dot_nt(a, b):
    return lax.dot_general(a, b, (((1,), (1,)), ((), ())), preferred_element_type=F32)


def _tree(f, xs):
    xs = list(xs)
    while len(xs) > 1:
        xs = [f(xs[i], xs[i + 1]) if i + 1 < len(xs) else xs[i] for i in range(0, len(xs), 2)]
    return xs[0]


def _mult(r, m):
    return r if isinstance(r, int) else pl.multiple_of(r, m)


def _step_order(H, dur_qk, dur_v, dur_a, lead, hold, fin_at, l_mm, l_sm, l_pin, vd, vgap, l_qs, l_pw):
    NG = H // G
    out = []
    t = 0
    nqk = nv = nwo = ns = npv = 0
    qk_end = [0] * H
    v_end = [0] * H
    s_end = [0] * NG
    pv_end = [0] * NG
    last = None
    fin_done = False
    npin = 0
    ends = {}
    while nwo < H:
        if not fin_done and t >= fin_at:
            out.append(("finish", 0))
            fin_done = True
        s_ok = ns < NG and nqk >= (ns + 1) * G and t >= qk_end[(ns + 1) * G - 1] + l_qs
        pv_ok = (npv < ns and nv >= (npv + 1) * G and t >= v_end[(npv + 1) * G - 1] + l_mm
                 and t >= s_end[npv] + l_sm)
        qk_ok = nqk < H
        v_ok = nv < H and (nqk >= H or nv + lead < nqk)
        wo_ok = (nwo < npv * G and t >= pv_end[nwo // G] + l_pw and (nv >= H or nwo + hold < nv))
        if s_ok:
            out.append(("s", ns)); t += dur_a[ns]; s_end[ns] = t; ns += 1
        elif pv_ok:
            out.append(("pv", npv)); t += dur_a[npv]; pv_end[npv] = t; npv += 1
        else:
            cand = [c for c, ok in (("qk", qk_ok), ("v", v_ok), ("wo", wo_ok)) if ok]
            if not cand:
                t += 4
                continue
            rot = {"qk": ("v", "wo", "qk"), "v": ("wo", "qk", "v"), "wo": ("qk", "v", "wo"),
                   None: ("qk", "v", "wo")}[last]
            c = [x for x in rot if x in cand][0]
            last = c
            if c in ("qk", "v") and npin < ns and t >= s_end[npin] + l_pin:
                while npin < ns and t >= s_end[npin] + l_pin:
                    out.append(("ppin", npin))
                    npin += 1
            if c == "qk":
                out.append(("qk", nqk)); t += dur_qk[nqk]; qk_end[nqk] = t; ends[("qk", nqk)] = t; nqk += 1
            elif c == "v":
                out.append(("v", nv)); t += dur_v[nv]; v_end[nv] = t; ends[("v", nv)] = t; nv += 1
            else:
                out.append(("wo", nwo)); t += 40; ends[("wo", nwo)] = t; nwo += 1
    if vd:
        tp = [0] * H
        for hd in range(H - 1, -1, -1):
            tp[hd] = ends[("wo", hd)] - 40 - vd
            if hd + 1 < H:
                tp[hd] = min(tp[hd], tp[hd + 1] - vgap[hd])
        after = {}
        for hd in range(H):
            cands = [key for key, e in ends.items() if e + 140 <= tp[hd] and e >= ends[("qk", hd)]]
            if cands:
                src = max(cands, key=lambda key: ends[key])
                after.setdefault(src, []).append(hd)
        out2 = []
        for op in out:
            out2.append(op)
            for hd in after.get(op, []):
                out2.append(("vs", (hd, op)))
        out = out2
    return out


def _kernel(x_hbm, mem0_ref, wq_hbm, wk_hbm, wv_hbm, wo_hbm, wr_ref, wg_hbm, wu_hbm, wd_hbm,
            out_hbm,
            x_ref, xs_ref, xp_scr, raw_scr, w_ref, wo_ref, wg_ref, wu_ref, wd_ref,
            pre_scr, xn_scr, xa_scr, xc_scr, xb_scr, ot_scr, pin_scr, out_v, ks_scr, vs_scr, pin2_scr, p_scr, zero_smem, sems,
            *, S, D, H, DH, M, F):
    L = M + SEG
    L0 = L - PR
    nseg = S // SEG
    HP = H // 2
    NC = D // DH
    NF = F // DH
    fill_heads_l = [list(range(H - NFILLS[li] * (US[li] - 1), H)) for li in range(2)]
    chain_fill = US[0] == US[1] and NFILLS[0] == NFILLS[1]
    scale = float(np.asarray(DH ** -0.5).astype(BF16))
    nvb = [NVB + (1 if hd in VB2 else 0) for hd in range(H)]
    koff = [8 + sum(M + 8 * n for n in nvb[:hd]) for hd in range(H)]

    NXC = 4
    xc = nseg // NXC
    HI = 4
    UP = 3
    NA = _env("NA", 3)
    NPRE = 2 * H
    NB = (NPRE - HI * (NA + 1)) // (2 * HI) - 1
    hb0 = HI * (NA + 1)
    pb0 = UP * (NA + 1)
    groups = [(0, 1), (1, 1), (2, 2), (4, 2)] + [(UP * it, UP) for it in range(2, NA + 1)]
    groups += [(pb0 + 2 * UP * it, 2 * UP) for it in range(NB)]
    groups += [(pb0 + 2 * UP * NB, 3 * HP - pb0 - 2 * UP * NB)]
    sem_xs, sem_x, sem_o, sem_o2, sem_xb, sem_wo, sem_ffn = 0, NXC, NXC + 1, NXC + 2, NXC + 3, NXC + 4, NXC + 5
    sem_w = NXC + 6

    for c in range(NXC):
        pltpu.make_async_copy(x_hbm.at[c * xc:(c + 1) * xc, SEG - PR:SEG, :],
                              xs_ref.at[c * xc:(c + 1) * xc], sems.at[sem_xs + c]).start()
    XA = US[0] + 1
    cp_xa = pltpu.make_async_copy(x_hbm.at[0:XA], x_ref.at[0:XA], sems.at[sem_x])
    cp_xb = pltpu.make_async_copy(x_hbm.at[XA:nseg], x_ref.at[XA:nseg], sems.at[sem_xb])
    X_AFTER = _env("X_AFTER", 30)
    w32 = [w.bitcast(U32) for w in (wq_hbm, wk_hbm, wv_hbm)]
    for gi, (g0, gn) in enumerate(groups):
        for i in range(g0, g0 + gn):
            pltpu.make_async_copy(w32[i // HP].at[:, i % HP, :], raw_scr.at[i], sems.at[sem_w + gi]).start()
            if i == X_AFTER:
                cp_xa.start()
    cp_wo = pltpu.make_async_copy(wo_hbm.bitcast(U32), wo_ref, sems.at[sem_wo])
    cp_wo.start()
    cp_xb.start()
    ffn_cps = [pltpu.make_async_copy(src.bitcast(U32), dst, sems.at[sem_ffn])
               for src, dst in ((wg_hbm, wg_ref), (wu_hbm, wu_ref), (wd_hbm, wd_ref))]
    if FFN_EARLY:
        for cp in ffn_cps:
            cp.start()
    zero_smem[0] = 0

    def wait_group(gi, g0, gn):
        blk = raw_scr.at[pl.ds(g0, gn)]
        pltpu.make_async_copy(blk, blk, sems.at[sem_w + gi]).wait()

    def unpack(i):
        for cb in range(D // 128):
            a = raw_scr[i, pl.ds(cb * 128, 64, stride=2), :]
            b = raw_scr[i, pl.ds(cb * 128 + 1, 64, stride=2), :]
            w_ref[2 * i, cb * 64:(cb + 1) * 64, :] = (a & jnp.uint32(0xFFFF)) | (b << 16)
            w_ref[2 * i + 1, cb * 64:(cb + 1) * 64, :] = (a >> 16) | (b & jnp.uint32(0xFFFF0000))

    def sel_rows(base, seg0, n):
        parts = []
        for u in range(n):
            r = _mult(base + (seg0 + u) * SEG + (SEG - PR), PR)
            parts.append(xn_scr[pl.ds(r, PR), :])
        return jnp.concatenate(parts, axis=0)

    def fill(li, i, lhs, prow):
        pre_scr[2 * H + i, pl.ds(prow, US[li] * PR), :] = _dot(lhs, _w(w_ref[2 * H + fill_heads_l[li][i]]))

    def ln_sel(c, carry):
        blk = xs_ref.at[pl.ds(c * xc, xc)]
        pltpu.make_async_copy(blk, blk, sems.at[sem_xs + c]).wait()
        xv = xs_ref[pl.ds(c * xc, xc)].astype(F32).reshape(xc * PR, D)
        xp_scr[pl.ds(pl.multiple_of(c * xc * PR, xc * PR), xc * PR), :] = _ln(xv).astype(BF16)
        return carry

    with _scope('p_ln'):
        lax.fori_loop(0, NXC, ln_sel, 0)
        pin_scr[...] = jnp.zeros_like(pin_scr)
        pin2_scr[...] = jnp.zeros_like(pin2_scr)
        p_scr[0:8, :] = jnp.zeros((8, DH), F32)
        for scr in (ks_scr, vs_scr):
            scr[0:8, :] = jnp.zeros((8, DH), F32)
        wait_group(0, *groups[0])
        unpack(0)

    def pre_wi(slot):
        nk = H // KS
        if isinstance(slot, int):
            return slot if slot < H else (H + KS * (slot - H) if slot < H + nk else 2 * H + slot - H - nk)
        return jnp.where(slot < H, slot, jnp.where(slot < H + nk, H + KS * (slot - H), H + slot - nk))

    pre_slot = {pre_wi(t): t for t in range(NPRE)}

    def pre_iter(hd0, nh, gi, g0, gn):
        wait_group(gi, g0, gn)
        xp = xp_scr[0:nseg * PR, :]
        pairs = [g0 + e for e in range(gn)]
        for e in range(nh):
            pre_scr[hd0 + e, 0:nseg * PR, :] = _dot(xp, _w(w_ref[pre_wi(hd0 + e)]))
            if e >= 1:
                take = -(-len(pairs) // (nh - e))
                for i in pairs[:take]:
                    unpack(i)
                pairs = pairs[take:]

    def pre_a(it, carry):
        pre_iter(HI * it, HI, 2 + it, UP * it, UP)
        return carry

    def pre_b(it, carry):
        pre_iter(hb0 + 2 * HI * it, 2 * HI, 3 + NA + it, pb0 + 2 * UP * it, 2 * UP)
        return carry

    dz = zero_smem[0]
    with _scope('p_0'):
        pre_iter(0, 2, 1, *groups[1])
        pre_iter(2, 2, 2, *groups[2])
        pre_iter(HI, HI, 3, groups[3][0] + dz, groups[3][1])
    with _scope('p_a'):
        lax.fori_loop(2, NA + 1, pre_a, 0)
    with _scope('p_b'):
        lax.fori_loop(0, NB, pre_b, 0)
    with _scope('p_last'):
        cp_xa.wait()
        pre_iter(hb0 + 2 * HI * NB, 2 * HI, len(groups) - 1, groups[-1][0] + dz, groups[-1][1])
        xn_scr[0:SEG, :] = _ln(x_ref[0].astype(F32))
        lhs0 = xp_scr[0:US[0] * PR, :]
        for i in range(len(fill_heads_l[0])):
            fill(0, i, lhs0, 0)
    with _scope('w_wo'):
        cp_wo.wait()
    if not FFN_EARLY:
        for cp in ffn_cps:
            cp.start()

    row = lax.broadcasted_iota(jnp.int32, (L, L), 0)
    col = lax.broadcasted_iota(jnp.int32, (L, L), 1)
    mask = (row < M) | (row >= col)
    wr = wr_ref[...].astype(F32).reshape(1, D)
    masks = {}
    for nb_ in set(nvb) - {0}:
        rr = lax.broadcasted_iota(jnp.int32, (L - 8 * nb_, L), 0)
        cc = lax.broadcasted_iota(jnp.int32, (L - 8 * nb_, L), 1)
        masks[nb_] = (rr < M) | (rr + 8 * nb_ >= cc)
    row8 = lax.broadcasted_iota(jnp.int32, (8, DH), 0)

    def vpu_offs(j):
        return list(range(0, M + 8 * j + 1)) + list(range(-1, -8, -1))

    def vpu_scores(hd, j, qb):
        b0 = koff[hd]
        qs = qb * (scale * LOG2E)
        ss = []
        for o_ in vpu_offs(j):
            sv = jnp.sum(qs * ks_scr[b0 + o_:b0 + o_ + 8, :], axis=-1, keepdims=True)
            sv = jnp.broadcast_to(sv, (8, DH))
            if o_ < 0:
                sv = jnp.where(row8 >= -o_, sv, -1e9 * LOG2E)
            ss.append(sv)
        return ss

    def vpu_pv(hd, j, ss, CH):
        b0 = koff[hd]
        offs = vpu_offs(j)
        mx = den = acc = None
        for c0 in range(0, len(offs), CH):
            cs = ss[c0:c0 + CH]
            cm = _tree(jnp.maximum, cs if mx is None else cs + [mx])
            if mx is not None:
                alpha = jnp.exp2(mx - cm)
                den = den * alpha
                acc = acc * alpha
            mx = cm
            if SERIAL:
                for sv, o_ in zip(cs, offs[c0:c0 + CH]):
                    pv = jnp.exp2(sv - mx)
                    t = pv * vs_scr[b0 + o_:b0 + o_ + 8, :]
                    den = pv if den is None else den + pv
                    acc = t if acc is None else acc + t
            else:
                ps = [jnp.exp2(sv - mx) for sv in cs]
                ts = [pv * vs_scr[b0 + o_:b0 + o_ + 8, :] for pv, o_ in zip(ps, offs[c0:c0 + CH])]
                den = _tree(jnp.add, ps if den is None else ps + [den])
                acc = _tree(jnp.add, ts if acc is None else ts + [acc])
        return acc * pl.reciprocal(den, approx=True)

    OB = US[1] * SEG

    def out_copy(r0, nrows, sem):
        return pltpu.make_async_copy(out_v.at[pl.ds(r0, nrows)], out_hbm.at[pl.ds(r0, nrows)], sems.at[sem])

    def layer(li):
        base = li * S
        first = li == 0
        U, NFILL, fill_heads = US[li], NFILLS[li], fill_heads_l[li]
        nblk = nseg // U
        dur_v = [32 if (hd in fill_heads or (first and 2 * H + hd in pre_slot)) else 40 for hd in range(H)]
        dur_qk = [(32 + (32 if H + hd in pre_slot else 40)) if first else 80 for hd in range(H)]
        sfx = "1" if first else "2"
        order = _step_order(H, dur_qk, dur_v, [L - 2 * sum(nvb[g * G:(g + 1) * G]) for g in range(H // G)],
                            _env("LEAD" + sfx, 28 if first else 32), _env("HOLD" + sfx, 9 if first else 12),
                            _env("FIN" + sfx, 2600 if first else 2000), _env("LMM" + sfx, 155 if first else 170), _env("LSM" + sfx, 450), _env("LPIN" + sfx, 450), _env("VD" + sfx, 0),
                            [_env("VGAP", 3) * (16 * nvb[hd] + 8 * (nvb[hd] > 1)) for hd in range(H)],
                            _env("LQS" + sfx, 250 if first else 140), _env("LPW" + sfx, 170 if first else 170))


        PIN_LAG = _env("PLAG" + sfx, 4)
        PIN_GAP = _env("PGAP" + sfx, 2)
        PIN_AT = sorted(set(list(range(PIN_LAG, H - PIN_GAP, _env("PSTEP" + sfx, 3 if first else 2))) + [H - PIN_GAP - 1]))
        CH = _env("CH" + sfx, 8 if first else 6)

        def finish(sp, o_tok, best_v, best_s, valid):
            r0 = _mult(sp * SEG, SEG)
            xin = x_ref[sp].astype(F32) if first else xb_scr[pl.ds(r0, SEG), :]
            x1 = _rb(xin + o_tok)
            xn1 = _ln(x1)
            r = _rb(jnp.sum(xn1 * wr, axis=-1, keepdims=True))
            upd = r > best_v
            if valid is not None:
                upd = jnp.logical_and(upd, valid)
            best_v = jnp.where(upd, r, best_v)
            best_s = jnp.where(upd, sp, best_s)
            x2 = _rb(x1 + xn1)
            xa_scr[pl.ds(r0, SEG), :] = x1
            if first:
                xc_scr[pl.ds(r0, SEG), :] = xn1
                xb_scr[pl.ds(r0, SEG), :] = x2
                xn_scr[pl.ds(S + r0, SEG), :] = _ln(x2)
            else:
                xn_scr[pl.ds(r0, SEG), :] = xn1
                out_v[pl.ds(r0, SEG), :] = x2.astype(BF16)
            return best_v, best_s

        def segment(s, mem, prev_tok, best_v, best_s, valid):
            r0 = pl.multiple_of(base + s * SEG, SEG)
            p0 = pl.multiple_of(s * PR, PR)
            hh = [jnp.concatenate([mem, xn_scr[pl.ds(r0, SEG), :]], axis=0)]
            hb = [hh[0][:L0].astype(BF16)]
            q = [None] * H
            k = [None] * H
            v = [None] * H
            p = [None] * H
            il = [None] * H
            o = [None] * H
            dd = [None] * H
            pw = [None] * H
            acc = None
            nacc = 0
            za = pl.multiple_of((s >> 12) * 8, 8)
            zb = pl.multiple_of((s >> 13) * 8, 8)

            ppin = [False]

            def proj(wi, pcol):
                lhs = hh[0]
                if ppin[0]:
                    ppin[0] = False
                    z = p_scr[0:8, :]
                    top = jnp.concatenate([lhs[:8, :DH] + z, lhs[:8, DH:]], axis=1)
                    lhs = jnp.concatenate([top, lhs[8:]], axis=0)
                if pcol is None:
                    return _dot(lhs, _w(w_ref[wi]))
                lb = hb[0] if (BFL & 1) and lhs is hh[0] else lhs[:L0]
                return jnp.concatenate(
                    [_dot(lb, _w(w_ref[wi])), pre_scr[pcol, pl.ds(p0, PR), :]], axis=0)

            for kind, i in order:
                if kind == "qk":
                    q[i] = proj(i, i if first else None)
                    k[i] = proj(H + i, pre_slot.get(H + i) if first else None)
                    if nvb[i]:
                        nk = M + 8 * nvb[i]
                        ks_scr[koff[i]:koff[i] + nk, :] = k[i][:nk]
                elif kind == "s":
                    for hd in range(i * G, (i + 1) * G):
                        qm = q[hd]
                        mk = mask
                        if nvb[hd]:
                            qm = jnp.concatenate([qm[:M], qm[M + 8 * nvb[hd]:]], axis=0)
                            mk = masks[nvb[hd]]
                        if (BFL & 2) and qm.shape[0] % 16 == 0:
                            qm = qm.astype(BF16)
                        sc = _dot_nt(qm, k[hd]) * (scale * LOG2E)
                        sc = jnp.where(mk, sc, -1e9 * LOG2E)
                        mx = jnp.max(sc, axis=-1, keepdims=True)
                        e = jnp.exp2(sc - mx)
                        pn = e * pl.reciprocal(jnp.sum(e, axis=-1, keepdims=True), approx=True)
                        if (BFL & 4) and pn.shape[0] % 16 == 0:
                            pn = pn.astype(BF16)
                        p[hd] = pn
                elif kind == "ppin":
                    if PPIN and p[i * G] is not None:
                        for hd in range(i * G, (i + 1) * G):
                            p_scr[pl.ds(za + 8 + hd * L, p[hd].shape[0]), 0:L] = p[hd]
                            p[hd] = None
                        ppin[0] = True
                elif kind == "v":
                    v[i] = proj(2 * H + i, 2 * H + fill_heads.index(i) if i in fill_heads
                                else (pre_slot.get(2 * H + i) if first else None))
                    if nvb[i]:
                        nk = M + 8 * nvb[i]
                        vs_scr[koff[i]:koff[i] + nk, :] = v[i][:nk]
                elif kind == "vs":
                    hd, (sk, si) = i
                    if nvb[hd]:
                        src = {"v": v, "wo": dd, "qk": k}[sk][si]
                        pin2_scr[pl.ds(za + 8, 8), :] = src[:8, :DH]
                        z = pin2_scr[pl.ds(zb, 8), :]
                        pw[hd] = [vpu_scores(hd, j, q[hd][M + 8 * j:M + 8 * (j + 1)] + z) for j in range(nvb[hd])]
                elif kind == "pv":
                    for hd in range(i * G, (i + 1) * G):
                        if p[hd] is None:
                            p[hd] = p_scr[8 + hd * L:8 + hd * L + L - 8 * nvb[hd], 0:L]
                        om = _dot(p[hd], v[hd])
                        p[hd] = None
                        o[hd] = om
                elif kind == "wo":
                    lhs = o[i]
                    if nvb[i]:
                        if pw[i] is None:
                            pw[i] = [vpu_scores(i, j, q[i][M + 8 * j:M + 8 * (j + 1)]) for j in range(nvb[i])]
                        ov = [vpu_pv(i, j, pw[i][j], CH) for j in range(nvb[i])]
                        lhs = jnp.concatenate([lhs[:M]] + ov + [lhs[M:]], axis=0)
                    if i - PIN_GAP in PIN_AT:
                        z = pin_scr[pl.ds(zb, 8), 0:DH]
                        lhs = jnp.concatenate([lhs[:8] + z, lhs[8:]], axis=0)
                    dd[i] = jnp.concatenate(
                        [_dot(lhs, _w(wo_ref[i * (DH // 2):(i + 1) * (DH // 2), c * DH:(c + 1) * DH])) for c in range(NC)],
                        axis=1)
                    if i in PIN_AT:
                        while nacc <= i - PIN_LAG:
                            acc = dd[nacc] if acc is None else acc + dd[nacc]
                            nacc += 1
                        pin_scr[pl.ds(za + 8, L), :] = acc
                elif kind == "finish":
                    sp = s - 1 if valid is None else jnp.maximum(s - 1, 0)
                    best_v, best_s = finish(sp, prev_tok, best_v, best_s, valid)
                    if first:
                        sn = jnp.minimum(s + 1, nseg - 1)
                        xn_scr[pl.ds(pl.multiple_of(sn * SEG, SEG), SEG), :] = _ln(x_ref[sn].astype(F32))
                    hh[0] = jnp.concatenate([mem, xn_scr[pl.ds(r0, SEG), :]], axis=0)
                    hb[0] = hh[0][:L0].astype(BF16)
            for j in range(nacc, H):
                acc = acc + dd[j]
            res = _rb(acc)
            return res[:M], res[M:], best_v, best_s

        def block(b, carry):
            mem, best_v, best_s = carry
            if first:
                @pl.when(b == 1)
                def _():
                    cp_xb.wait()
            else:
                @pl.when(b >= 2)
                def _():
                    out_copy(pl.multiple_of((b - 2) * OB, OB), OB, sem_o).start()
            tok = ot_scr[...]
            nb = jnp.minimum(b + 1, nblk - 1)
            for u in range(U):
                s = b * U + u
                mem, tok, best_v, best_s = segment(s, mem, tok, best_v, best_s, (s > 0) if u == 0 else None)
                if u < U - 1:
                    prow = (b + 1) * U * PR
                    if first:
                        lhs = xp_scr[pl.ds(pl.multiple_of(nb * U * PR, U * PR), U * PR), :]
                        if chain_fill:
                            lhs = jnp.where(b == nblk - 1, sel_rows(S, 0, U).astype(BF16), lhs)
                            prow = jnp.where(b == nblk - 1, 0, prow)
                    else:
                        lhs = sel_rows(base, nb * U, U).astype(BF16)
                    for i in range(u * NFILL, (u + 1) * NFILL):
                        fill(li, i, lhs, pl.multiple_of(prow, U * PR))
            ot_scr[...] = tok
            return mem, best_v, best_s

        ot_scr[...] = jnp.zeros_like(ot_scr)
        init = (mem0_ref[...].astype(F32),
                jnp.full((SEG, 1), -jnp.inf, F32),
                jnp.zeros((SEG, 1), jnp.int32))
        with _scope('main%d' % li):
            _, best_v, best_s = lax.fori_loop(0, nblk, block, init)
        if first:
            for cp in ffn_cps:
                cp.wait()
        best_v, best_s = finish(nseg - 1, ot_scr[...], best_v, best_s, None)
        if not first:
            out_copy((nblk - 2) * OB, 2 * OB, sem_o).start()

        vmax = jnp.max(best_v, axis=0, keepdims=True)
        tok = best_s * SEG + lax.broadcasted_iota(jnp.int32, (SEG, 1), 0)
        idx = jnp.min(jnp.where(best_v == vmax, tok, S))
        idx = jnp.clip(idx, 0, S - 1)
        xs = xc_scr[pl.ds(idx, 1), :] if first else xn_scr[pl.ds(idx, 1), :]
        x1 = xa_scr[pl.ds(idx, 1), :]
        xs8 = jnp.broadcast_to(xs, (8, D))
        g = _rb(_dot(xs8, _w(wg_ref[...])))
        u = _rb(_dot(xs8, _w(wu_ref[...])))
        g = _rb(g * _rb(jax.nn.sigmoid(g)))
        gu = _rb(g * u)
        y = _rb(_dot(gu, _w(wd_ref[...])))
        y = _rb(y * _rb(jax.nn.sigmoid(vmax)))
        new = _rb(x1 + _rb(xs + y[0:1]))
        return idx, new

    idx, new = layer(0)
    xb_scr[pl.ds(idx, 1), :] = new
    xn_scr[pl.ds(S + idx, 1), :] = _ln(new)

    def fill_first():
        lhs0 = sel_rows(S, 0, US[1]).astype(BF16)
        for i in range(len(fill_heads_l[1])):
            fill(1, i, lhs0, 0)

    if chain_fill:
        pl.when(idx < US[1] * SEG)(fill_first)
    else:
        fill_first()

    idx, new = layer(1)
    out_copy(0, S, sem_o).wait()
    b0 = pl.multiple_of((idx // 16) * 16, 16)
    blk = out_v[pl.ds(b0, 16), :].astype(F32)
    rid = b0 + lax.broadcasted_iota(jnp.int32, (16, D), 0)
    out_v[pl.ds(b0, 16), :] = jnp.where(rid == idx, new, blk).astype(BF16)
    cp = out_copy(b0, 16, sem_o2)
    cp.start()
    cp.wait()


@jax.jit
def pallas_interleave_layers__memory_aug_recurrent_mem_tr__moe_arch_mod__prompt_kernel(
    A_x, A_mem0, A_Wq, A_Wk, A_Wv, A_Wo, A_seg_len, B_x, B_w_r, B_w_gate, B_w_up, B_w_down,
):
    B, S, D = A_x.shape
    _, H, DH = A_Wq.shape
    M = A_mem0.shape[1]
    F = B_w_gate.shape[1]
    assert B == 1 and S % (SEG * max(US)) == 0
    nseg = S // SEG
    kern = functools.partial(_kernel, S=S, D=D, H=H, DH=DH, M=M, F=F)
    hbm = pl.BlockSpec(memory_space=pl.ANY)
    vm = pl.BlockSpec(memory_space=pltpu.VMEM)
    nsem = 22
    out = pl.pallas_call(
        kern,
        out_shape=jax.ShapeDtypeStruct((S, D), BF16),
        in_specs=[hbm, vm, hbm, hbm, hbm, hbm, vm, hbm, hbm, hbm],
        out_specs=hbm,
        scratch_shapes=[
            pltpu.VMEM((nseg, SEG, D), BF16),
            pltpu.VMEM((nseg, PR, D), BF16),
            pltpu.VMEM((nseg * PR, D), BF16),
            pltpu.VMEM((3 * (H // 2), D, DH), U32),
            pltpu.VMEM((3 * H, D // 2, DH), U32),
            pltpu.VMEM((H * DH // 2, D), U32),
            pltpu.VMEM((D // 2, F), U32), pltpu.VMEM((D // 2, F), U32),
            pltpu.VMEM((F // 2, D), U32),
            pltpu.VMEM((2 * H + max(n * (u - 1) for n, u in zip(NFILLS, US)), (nseg + max(US)) * PR, DH), F32),
            pltpu.VMEM((2 * S, D), F32),
            pltpu.VMEM((S, D), F32), pltpu.VMEM((S, D), F32), pltpu.VMEM((S, D), F32),
            pltpu.VMEM((SEG, D), F32),
            pltpu.VMEM((M + SEG + 8, D), F32),
            pltpu.VMEM((S, D), BF16),
            pltpu.VMEM((8 + H * (M + 16), DH), F32), pltpu.VMEM((8 + H * (M + 16), DH), F32),
            pltpu.VMEM((16, DH), F32),
            pltpu.VMEM((8 + H * (M + SEG), DH), F32),
            pltpu.SMEM((1,), jnp.int32),
            pltpu.SemaphoreType.DMA((nsem,))],
        compiler_params=pltpu.CompilerParams(vmem_limit_bytes=110 * 1024 * 1024),
    )(A_x.reshape(nseg, SEG, D), A_mem0.reshape(M, D), A_Wq, A_Wk, A_Wv,
      A_Wo.reshape(H * DH, D), B_w_r, B_w_gate, B_w_up, B_w_down)
    return out.reshape(B, S, D)
```

```python
import functools

import numpy as np
import jax
import jax.numpy as jnp
from jax import lax
import jax.experimental.pallas as pl
import jax.experimental.pallas.tpu as pltpu

F32 = jnp.float32
BF16 = jnp.bfloat16
U32 = jnp.uint32
SEG = 32
EPS = 1e-05
LOG2E = 1.4426950408889634
G = 4
PR = 8
VB = 8
U = 4
NFILL = 4

TUNE = (
    dict(lead=28, hold=9, fin=2600, l_vp=155, l_sp=450, l_qs=250, l_pw=170, plag=4, pgap=2, pstep=3, ch=8),
    dict(lead=32, hold=12, fin=2000, l_vp=170, l_sp=450, l_qs=140, l_pw=170, plag=4, pgap=2, pstep=2, ch=6),
)


def _rb(x):
    return x.astype(BF16).astype(F32)


def _ln(x):
    d = x.shape[-1]
    mu = jnp.sum(x, axis=-1, keepdims=True) * (1.0 / d)
    c = x - mu
    var = jnp.sum(c * c, axis=-1, keepdims=True) * (1.0 / d)
    m = _rb(mu)
    v = _rb(var)
    den = _rb(jnp.sqrt(_rb(v + EPS)))
    return _rb(_rb(x - m) / den)


def _w(x):
    return pltpu.bitcast(x, BF16)


def _dot(a, b):
    return lax.dot_general(a, b, (((1,), (0,)), ((), ())), preferred_element_type=F32)


def _dot_nt(a, b):
    return lax.dot_general(a, b, (((1,), (1,)), ((), ())), preferred_element_type=F32)


def _tree(f, xs):
    xs = list(xs)
    while len(xs) > 1:
        xs = [f(xs[i], xs[i + 1]) if i + 1 < len(xs) else xs[i] for i in range(0, len(xs), 2)]
    return xs[0]


def _mult(r, m):
    return r if isinstance(r, int) else pl.multiple_of(r, m)


def _step_order(H, dur_qk, dur_v, dur_a, dur_wo, t_):
    NG = H // G
    out = []
    t = 0
    nqk = nv = nwo = ns = npv = 0
    qk_end, v_end, s_end, pv_end = [0] * H, [0] * H, [0] * NG, [0] * NG
    last = None
    fin_done = False
    while nwo < H:
        if not fin_done and t >= t_["fin"]:
            out.append(("finish", 0))
            fin_done = True
        s_ok = ns < NG and nqk >= (ns + 1) * G and t >= qk_end[(ns + 1) * G - 1] + t_["l_qs"]
        pv_ok = (npv < ns and nv >= (npv + 1) * G and t >= v_end[(npv + 1) * G - 1] + t_["l_vp"]
                 and t >= s_end[npv] + t_["l_sp"])
        qk_ok = nqk < H
        v_ok = nv < H and (nqk >= H or nv + t_["lead"] < nqk)
        wo_ok = (nwo < npv * G and t >= pv_end[nwo // G] + t_["l_pw"]
                 and (nv >= H or nwo + t_["hold"] < nv))
        if s_ok:
            out.append(("s", ns))
            t += dur_a
            s_end[ns] = t
            ns += 1
        elif pv_ok:
            out.append(("pv", npv))
            t += dur_a
            pv_end[npv] = t
            npv += 1
        else:
            cand = [c for c, ok in (("qk", qk_ok), ("v", v_ok), ("wo", wo_ok)) if ok]
            if not cand:
                t += 4
                continue
            rot = {"qk": ("v", "wo", "qk"), "v": ("wo", "qk", "v"), "wo": ("qk", "v", "wo"),
                   None: ("qk", "v", "wo")}[last]
            last = [c for c in rot if c in cand][0]
            if last == "qk":
                out.append(("qk", nqk))
                t += dur_qk
                qk_end[nqk] = t
                nqk += 1
            elif last == "v":
                out.append(("v", nv))
                t += dur_v[nv]
                v_end[nv] = t
                nv += 1
            else:
                out.append(("wo", nwo))
                t += dur_wo
                nwo += 1
    return out


NXC = 4
HI = 4
UP = 3
NA, NB = 2, 5
HA0, PA0 = 10, 7
HB0, PB0 = HA0 + HI * NA, PA0 + UP * NA


def _groups(npairs):
    g = [(0, 1), (1, 2), (3, 2), (5, 2)] + [(PA0 + UP * it, UP) for it in range(NA)]
    g += [(PB0 + 2 * UP * it, 2 * UP) for it in range(NB)]
    g += [(PB0 + 2 * UP * NB, npairs - PB0 - 2 * UP * NB)]
    return g


SEM_XS, SEM_X, SEM_O, SEM_O2, SEM_XB, SEM_WO, SEM_FFN, SEM_W = 0, 4, 5, 6, 7, 8, 9, 10


def _kernel(x_hbm, mem0_hbm, wq_hbm, wk_hbm, wv_hbm, wo_hbm, wr_hbm, wg_hbm, wu_hbm, wd_hbm,
            out_hbm,
            x_ref, xs_ref, xp_scr, raw_scr, w_ref, wo_ref, wg_ref, wu_ref, wd_ref,
            pre_scr, xn_scr, xa_scr, xc_scr, xb_scr, ot_scr, pin_scr, out_v, ks_scr, vs_scr,
            mem0_ref, wr_ref, zero_smem, sems,
            *, S, D, H, DH, M):
    L = M + SEG
    L0 = L - PR
    LM = L - VB
    KV = M + VB
    nseg = S // SEG
    nblk = nseg // U
    HP = H // 2
    NC = D // DH
    NPRE = 2 * H
    NFH = NFILL * (U - 1)
    fill_heads = list(range(H - NFH, H))
    xc = nseg // NXC
    groups = _groups(3 * HP)
    qscale = float(np.asarray(DH ** -0.5).astype(BF16)) * LOG2E
    neg = -1e9 * LOG2E

    def start_xs(c):
        pltpu.make_async_copy(x_hbm.at[c * xc:(c + 1) * xc, SEG - PR:SEG, :],
                              xs_ref.at[c * xc:(c + 1) * xc], sems.at[SEM_XS + min(c, 2)]).start()

    start_xs(0)
    start_xs(1)
    XA = U + 1
    early_cps = [pltpu.make_async_copy(x_hbm.at[0:XA], x_ref.at[0:XA], sems.at[SEM_X]),
                 pltpu.make_async_copy(mem0_hbm, mem0_ref, sems.at[SEM_X]),
                 pltpu.make_async_copy(wr_hbm, wr_ref, sems.at[SEM_X])]
    cp_xb = pltpu.make_async_copy(x_hbm.at[XA:nseg], x_ref.at[XA:nseg], sems.at[SEM_XB])
    w32 = [w.bitcast(U32) for w in (wq_hbm, wk_hbm, wv_hbm)]
    for gi, (g0, gn) in enumerate(groups):
        for i in range(g0, g0 + gn):
            pltpu.make_async_copy(w32[i // HP].at[:, i % HP, :], raw_scr.at[i], sems.at[SEM_W + gi]).start()
            if i == 0:
                start_xs(2)
                start_xs(3)
            if i == 30:
                for cp in early_cps:
                    cp.start()
    cp_wo = pltpu.make_async_copy(wo_hbm.bitcast(U32), wo_ref, sems.at[SEM_WO])
    cp_wo.start()
    cp_xb.start()
    ffn_cps = [pltpu.make_async_copy(src.bitcast(U32), dst, sems.at[SEM_FFN])
               for src, dst in ((wg_hbm, wg_ref), (wu_hbm, wu_ref), (wd_hbm, wd_ref))]
    for cp in ffn_cps:
        cp.start()
    zero_smem[0] = 0

    def wait_group(gi, g0, gn):
        blk = raw_scr.at[pl.ds(g0, gn)]
        pltpu.make_async_copy(blk, blk, sems.at[SEM_W + gi]).wait()

    def unpack(i):
        for cb in range(D // 128):
            a = raw_scr[i, pl.ds(cb * 128, 64, stride=2), :]
            b = raw_scr[i, pl.ds(cb * 128 + 1, 64, stride=2), :]
            w_ref[2 * i, cb * 64:(cb + 1) * 64, :] = (a & jnp.uint32(0xFFFF)) | (b << 16)
            w_ref[2 * i + 1, cb * 64:(cb + 1) * 64, :] = (a >> 16) | (b & jnp.uint32(0xFFFF0000))

    def sel_rows(seg0):
        parts = [xn_scr[pl.ds(_mult(S + (seg0 + u) * SEG + (SEG - PR), PR), PR), :] for u in range(U)]
        return jnp.concatenate(parts, axis=0).astype(BF16)

    def fill(i, lhs, prow):
        pre_scr[NPRE + i, pl.ds(prow, U * PR), :] = _dot(lhs, _w(w_ref[2 * H + fill_heads[i]]))

    def wait_xs(c, n):
        blk = xs_ref.at[pl.ds(c * xc, n * xc)]
        pltpu.make_async_copy(blk, blk, sems.at[SEM_XS + c]).wait()

    def ln_sel(c):
        xv = xs_ref[pl.ds(c * xc, xc)].astype(F32).reshape(xc * PR, D)
        xp_scr[pl.ds(_mult(c * xc * PR, xc * PR), xc * PR), :] = _ln(xv).astype(BF16)

    def ln_body(c, carry):
        wait_xs(c, 1)
        ln_sel(c)
        return carry

    lax.fori_loop(0, 2, ln_body, 0)
    pin_scr[...] = jnp.zeros_like(pin_scr)
    for scr in (ks_scr, vs_scr):
        scr[0:8, :] = jnp.zeros((8, DH), F32)
    for u in range(U):
        r = S + u * SEG + (SEG - PR)
        xn_scr[r:r + PR, :] = jnp.zeros((PR, D), F32)
    wait_group(0, *groups[0])
    unpack(0)
    wait_xs(2, 2)
    half = 2 * xc * PR
    for e in range(2):
        pre_scr[e, 0:half, :] = _dot(xp_scr[0:half, :], _w(w_ref[e]))
    ln_sel(2)
    ln_sel(3)
    for e in range(2):
        pre_scr[e, half:2 * half, :] = _dot(xp_scr[half:2 * half, :], _w(w_ref[e]))

    def pre_iter(hd0, nh, gi, g0, gn, now=0):
        wait_group(gi, g0, gn)
        xp = xp_scr[...]
        pairs = [g0 + e for e in range(gn)]
        for i in pairs[:now]:
            unpack(i)
        pairs = pairs[now:]
        for e in range(nh):
            pre_scr[hd0 + e, 0:nseg * PR, :] = _dot(xp, _w(w_ref[hd0 + e]))
            if e >= 1:
                take = -(-len(pairs) // (nh - e))
                for i in pairs[:take]:
                    unpack(i)
                pairs = pairs[take:]

    def pre_a(it, carry):
        pre_iter(HA0 + HI * it, HI, 4 + it, PA0 + UP * it, UP)
        return carry

    def pre_b(it, carry):
        pre_iter(HB0 + 2 * HI * it, 2 * HI, 4 + NA + it, PB0 + 2 * UP * it, 2 * UP)
        return carry

    dz = zero_smem[0]
    pre_iter(2, 2, 1, groups[1][0] + dz, groups[1][1], now=1)
    pre_iter(4, 2, 2, groups[2][0] + dz, groups[2][1])
    pre_iter(6, HI, 3, groups[3][0] + dz, groups[3][1])
    lax.fori_loop(0, NA, pre_a, 0)
    lax.fori_loop(0, NB, pre_b, 0)
    for cp in early_cps:
        cp.wait()
    pre_iter(HB0 + 2 * HI * NB, NPRE - HB0 - 2 * HI * NB, len(groups) - 1, groups[-1][0] + dz, groups[-1][1])
    xn_scr[0:SEG, :] = _ln(x_ref[0].astype(F32))
    lhs0 = xp_scr[0:U * PR, :]
    for i in range(NFH):
        fill(i, lhs0, 0)
    cp_wo.wait()

    wr = wr_ref[...].astype(F32).reshape(1, D)
    rr = lax.broadcasted_iota(jnp.int32, (LM, L), 0)
    cc = lax.broadcasted_iota(jnp.int32, (LM, L), 1)
    mask = (rr < M) | (rr + VB >= cc)
    row8 = lax.broadcasted_iota(jnp.int32, (VB, DH), 0)
    shifts = list(range(0, M + 1)) + list(range(-1, -VB, -1))

    def vpu_attention(hd, qb, ch):
        b0 = 8 + KV * hd
        qs = qb * qscale
        ss = []
        for o in shifts:
            sv = jnp.sum(qs * ks_scr[b0 + o:b0 + o + VB, :], axis=-1, keepdims=True)
            sv = jnp.broadcast_to(sv, (VB, DH))
            if o < 0:
                sv = jnp.where(row8 >= -o, sv, neg)
            ss.append(sv)
        mx = den = acc = None
        for c0 in range(0, len(shifts), ch):
            cs = ss[c0:c0 + ch]
            cm = _tree(jnp.maximum, cs if mx is None else cs + [mx])
            if mx is not None:
                alpha = jnp.exp2(mx - cm)
                den = den * alpha
                acc = acc * alpha
            mx = cm
            for sv, o in zip(cs, shifts[c0:c0 + ch]):
                pv = jnp.exp2(sv - mx)
                t = pv * vs_scr[b0 + o:b0 + o + VB, :]
                den = pv if den is None else den + pv
                acc = t if acc is None else acc + t
        return acc * pl.reciprocal(den, approx=True)

    OB = U * SEG

    def out_copy(r0, nrows, sem):
        return pltpu.make_async_copy(out_v.at[pl.ds(r0, nrows)], out_hbm.at[pl.ds(r0, nrows)], sems.at[sem])

    def layer(li):
        first = li == 0
        base = li * S
        t_ = TUNE[li]
        order = _step_order(H, 2 * (L0 if first else L), [L0 if hd in fill_heads else L for hd in range(H)],
                            LM, L, t_)
        plag, pgap = t_["plag"], t_["pgap"]
        pin_at = sorted(set(list(range(plag, H - pgap, t_["pstep"])) + [H - pgap - 1]))

        def finish(sp, o_tok, best_v, best_s, valid):
            r0 = _mult(sp * SEG, SEG)
            xin = x_ref[sp].astype(F32) if first else xb_scr[pl.ds(r0, SEG), :]
            x1 = _rb(xin + o_tok)
            xn1 = _ln(x1)
            r = _rb(jnp.sum(xn1 * wr, axis=-1, keepdims=True))
            upd = r > best_v
            if valid is not None:
                upd = jnp.logical_and(upd, valid)
            best_v = jnp.where(upd, r, best_v)
            best_s = jnp.where(upd, sp, best_s)
            x2 = _rb(x1 + xn1)
            xa_scr[pl.ds(r0, SEG), :] = x1
            if first:
                xc_scr[pl.ds(r0, SEG), :] = xn1
                xb_scr[pl.ds(r0, SEG), :] = x2
                xn_scr[pl.ds(S + r0, SEG), :] = _ln(x2)
            else:
                xn_scr[pl.ds(r0, SEG), :] = xn1
                out_v[pl.ds(r0, SEG), :] = x2.astype(BF16)
            return best_v, best_s

        def segment(s, mem, prev_tok, best_v, best_s, valid):
            r0 = pl.multiple_of(base + s * SEG, SEG)
            p0 = pl.multiple_of(s * PR, PR)
            h = jnp.concatenate([mem, xn_scr[pl.ds(r0, SEG), :]], axis=0)
            hb = h[:L0].astype(BF16)
            q, k, v, p, o, dd = ([None] * H for _ in range(6))
            acc = None
            nacc = 0
            za = pl.multiple_of((s >> 12) * 8, 8)
            zb = pl.multiple_of((s >> 13) * 8, 8)

            def proj(wi, slot):
                if slot is None:
                    return _dot(h, _w(w_ref[wi]))
                return jnp.concatenate([_dot(hb, _w(w_ref[wi])), pre_scr[slot, pl.ds(p0, PR), :]], axis=0)

            for kind, i in order:
                if kind == "qk":
                    q[i] = proj(i, i if first else None)
                    k[i] = proj(H + i, H + i if first else None)
                    ks_scr[8 + KV * i:8 + KV * (i + 1), :] = k[i][:KV]
                elif kind == "s":
                    for hd in range(i * G, (i + 1) * G):
                        qm = jnp.concatenate([q[hd][:M], q[hd][KV:]], axis=0)
                        sc = jnp.where(mask, _dot_nt(qm, k[hd]) * qscale, neg)
                        e = jnp.exp2(sc - jnp.max(sc, axis=-1, keepdims=True))
                        pn = e * pl.reciprocal(jnp.sum(e, axis=-1, keepdims=True), approx=True)
                        p[hd] = pn.astype(BF16)
                elif kind == "v":
                    v[i] = proj(2 * H + i, NPRE + fill_heads.index(i) if i in fill_heads else None)
                    vs_scr[8 + KV * i:8 + KV * (i + 1), :] = v[i][:KV]
                elif kind == "pv":
                    for hd in range(i * G, (i + 1) * G):
                        o[hd] = _dot(p[hd], v[hd])
                elif kind == "wo":
                    ov = vpu_attention(i, q[i][M:KV], t_["ch"])
                    top = o[i][:M]
                    if i - pgap in pin_at:
                        top = top + pin_scr[pl.ds(zb, 8), 0:DH]
                    lhs = jnp.concatenate([top, ov, o[i][M:]], axis=0)
                    dd[i] = jnp.concatenate(
                        [_dot(lhs, _w(wo_ref[i * (DH // 2):(i + 1) * (DH // 2), c * DH:(c + 1) * DH]))
                         for c in range(NC)], axis=1)
                    if i in pin_at:
                        while nacc <= i - plag:
                            acc = dd[nacc] if acc is None else acc + dd[nacc]
                            nacc += 1
                        pin_scr[pl.ds(za + 8, L), :] = acc
                else:
                    sp = s - 1 if valid is None else jnp.maximum(s - 1, 0)
                    best_v, best_s = finish(sp, prev_tok, best_v, best_s, valid)
                    if first:
                        sn = jnp.minimum(s + 1, nseg - 1)
                        xn_scr[pl.ds(pl.multiple_of(sn * SEG, SEG), SEG), :] = _ln(x_ref[sn].astype(F32))
                    h = jnp.concatenate([mem, xn_scr[pl.ds(r0, SEG), :]], axis=0)
                    hb = h[:L0].astype(BF16)
            for j in range(nacc, H):
                acc = acc + dd[j]
            res = _rb(acc)
            return res[:M], res[M:], best_v, best_s

        def block(b, carry):
            mem, best_v, best_s = carry
            if first:
                @pl.when(b == 1)
                def _():
                    cp_xb.wait()
            else:
                @pl.when(b >= 2)
                def _():
                    out_copy(pl.multiple_of((b - 2) * OB, OB), OB, SEM_O).start()
            tok = ot_scr[...]
            nb = jnp.minimum(b + 1, nblk - 1)
            for u in range(U):
                s = b * U + u
                mem, tok, best_v, best_s = segment(s, mem, tok, best_v, best_s, (s > 0) if u == 0 else None)
                if u < U - 1:
                    prow = (b + 1) * U * PR
                    if first:
                        lhs = xp_scr[pl.ds(pl.multiple_of(nb * U * PR, U * PR), U * PR), :]
                        lhs = jnp.where(b == nblk - 1, sel_rows(0), lhs)
                        prow = jnp.where(b == nblk - 1, 0, prow)
                    else:
                        lhs = sel_rows(nb * U)
                    for i in range(u * NFILL, (u + 1) * NFILL):
                        fill(i, lhs, pl.multiple_of(prow, U * PR))
            ot_scr[...] = tok
            return mem, best_v, best_s

        ot_scr[...] = jnp.zeros_like(ot_scr)
        init = (mem0_ref[...].astype(F32),
                jnp.full((SEG, 1), -jnp.inf, F32),
                jnp.zeros((SEG, 1), jnp.int32))
        _, best_v, best_s = lax.fori_loop(0, nblk, block, init)
        if first:
            for cp in ffn_cps:
                cp.wait()
        best_v, best_s = finish(nseg - 1, ot_scr[...], best_v, best_s, None)
        if not first:
            out_copy((nblk - 2) * OB, 2 * OB, SEM_O).start()

        vmax = jnp.max(best_v, axis=0, keepdims=True)
        tok = best_s * SEG + lax.broadcasted_iota(jnp.int32, (SEG, 1), 0)
        idx = jnp.min(jnp.where(best_v == vmax, tok, S))
        idx = jnp.clip(idx, 0, S - 1)
        xs = xc_scr[pl.ds(idx, 1), :] if first else xn_scr[pl.ds(idx, 1), :]
        x1 = xa_scr[pl.ds(idx, 1), :]
        xs8 = jnp.broadcast_to(xs, (8, D))
        g = _rb(_dot(xs8, _w(wg_ref[...])))
        u = _rb(_dot(xs8, _w(wu_ref[...])))
        g = _rb(g * _rb(jax.nn.sigmoid(g)))
        y = _rb(_dot(_rb(g * u), _w(wd_ref[...])))
        y = _rb(y * _rb(jax.nn.sigmoid(vmax)))
        return idx, _rb(x1 + _rb(xs + y[0:1]))

    idx, new = layer(0)
    xb_scr[pl.ds(idx, 1), :] = new
    xn_scr[pl.ds(S + idx, 1), :] = _ln(new)

    @pl.when(idx < U * SEG)
    def _():
        lhs = sel_rows(0)
        for i in range(NFH):
            fill(i, lhs, 0)

    idx, new = layer(1)
    out_copy(0, S, SEM_O).wait()
    b0 = pl.multiple_of((idx // 16) * 16, 16)
    blk = out_v[pl.ds(b0, 16), :].astype(F32)
    rid = b0 + lax.broadcasted_iota(jnp.int32, (16, D), 0)
    out_v[pl.ds(b0, 16), :] = jnp.where(rid == idx, new, blk).astype(BF16)
    cp = out_copy(b0, 16, SEM_O2)
    cp.start()
    cp.wait()


@jax.jit
def pallas_interleave_layers__memory_aug_recurrent_mem_tr__moe_arch_mod__prompt_kernel(
    A_x, A_mem0, A_Wq, A_Wk, A_Wv, A_Wo, A_seg_len, B_x, B_w_r, B_w_gate, B_w_up, B_w_down,
):
    B, S, D = A_x.shape
    _, H, DH = A_Wq.shape
    M = A_mem0.shape[1]
    F = B_w_gate.shape[1]
    assert (B, S, D, H, DH, M) == (1, 2048, 512, 32, 128, 8)
    nseg = S // SEG
    kern = functools.partial(_kernel, S=S, D=D, H=H, DH=DH, M=M)
    hbm = pl.BlockSpec(memory_space=pl.ANY)
    out = pl.pallas_call(
        kern,
        out_shape=jax.ShapeDtypeStruct((S, D), BF16),
        in_specs=[hbm] * 10,
        out_specs=hbm,
        scratch_shapes=[
            pltpu.VMEM((nseg, SEG, D), BF16),
            pltpu.VMEM((nseg, PR, D), BF16),
            pltpu.VMEM((nseg * PR, D), BF16),
            pltpu.VMEM((3 * (H // 2), D, DH), U32),
            pltpu.VMEM((3 * H, D // 2, DH), U32),
            pltpu.VMEM((H * DH // 2, D), U32),
            pltpu.VMEM((D // 2, F), U32), pltpu.VMEM((D // 2, F), U32), pltpu.VMEM((F // 2, D), U32),
            pltpu.VMEM((2 * H + NFILL * (U - 1), (nseg + U) * PR, DH), F32),
            pltpu.VMEM((2 * S, D), F32),
            pltpu.VMEM((S, D), F32), pltpu.VMEM((S, D), F32), pltpu.VMEM((S, D), F32),
            pltpu.VMEM((SEG, D), F32),
            pltpu.VMEM((M + SEG + 8, D), F32),
            pltpu.VMEM((S, D), BF16),
            pltpu.VMEM((8 + H * (M + VB), DH), F32), pltpu.VMEM((8 + H * (M + VB), DH), F32),
            pltpu.VMEM((M, D), BF16), pltpu.VMEM((D,), BF16),
            pltpu.SMEM((1,), jnp.int32),
            pltpu.SemaphoreType.DMA((SEM_W + len(_groups(3 * (H // 2))),))],
        compiler_params=pltpu.CompilerParams(vmem_limit_bytes=110 * 1024 * 1024),
    )(A_x.reshape(nseg, SEG, D), A_mem0.reshape(M, D), A_Wq, A_Wk, A_Wv,
      A_Wo.reshape(H * DH, D), B_w_r, B_w_gate, B_w_up, B_w_down)
    return out.reshape(B, S, D)
```

```python
import functools

import numpy as np
import jax
import jax.numpy as jnp
from jax import lax
import jax.experimental.pallas as pl
import jax.experimental.pallas.tpu as pltpu

F32 = jnp.float32
BF16 = jnp.bfloat16
U32 = jnp.uint32
SEG = 32
EPS = 1e-05
LOG2E = 1.4426950408889634
G = 4
PR = 8
VB = 8
U = 4
NFILL = 4
NP2 = 2

TUNE = (
    dict(lead=28, hold=9, fin=2600, l_vp=155, l_sp=450, l_qs=250, l_pw=170, plag=4, pgap=2, pstep=3, ch=8),
    dict(lead=32, hold=12, fin=2000, l_vp=170, l_sp=450, l_qs=140, l_pw=170, plag=4, pgap=2, pstep=2, ch=6),
)


def _rb(x):
    return x.astype(BF16).astype(F32)


def _ln(x):
    d = x.shape[-1]
    mu = jnp.sum(x, axis=-1, keepdims=True) * (1.0 / d)
    c = x - mu
    var = jnp.sum(c * c, axis=-1, keepdims=True) * (1.0 / d)
    m = _rb(mu)
    v = _rb(var)
    den = _rb(jnp.sqrt(_rb(v + EPS)))
    return _rb(_rb(x - m) / den)


def _w(x):
    return pltpu.bitcast(x, BF16)


def _dot(a, b):
    return lax.dot_general(a, b, (((1,), (0,)), ((), ())), preferred_element_type=F32)


def _dot_nt(a, b):
    return lax.dot_general(a, b, (((1,), (1,)), ((), ())), preferred_element_type=F32)


def _tree(f, xs):
    xs = list(xs)
    while len(xs) > 1:
        xs = [f(xs[i], xs[i + 1]) if i + 1 < len(xs) else xs[i] for i in range(0, len(xs), 2)]
    return xs[0]


def _mult(r, m):
    return r if isinstance(r, int) else pl.multiple_of(r, m)


def _step_order(H, dur_qk, dur_v, dur_a, dur_wo, t_):
    NG = H // G
    out = []
    t = 0
    nqk = nv = nwo = ns = npv = 0
    qk_end, v_end, s_end, pv_end = [0] * H, [0] * H, [0] * NG, [0] * NG
    last = None
    fin_done = False
    while nwo < H:
        if not fin_done and t >= t_["fin"]:
            out.append(("finish", 0))
            fin_done = True
        s_ok = ns < NG and nqk >= (ns + 1) * G and t >= qk_end[(ns + 1) * G - 1] + t_["l_qs"]
        pv_ok = (npv < ns and nv >= (npv + 1) * G and t >= v_end[(npv + 1) * G - 1] + t_["l_vp"]
                 and t >= s_end[npv] + t_["l_sp"])
        qk_ok = nqk < H
        v_ok = nv < H and (nqk >= H or nv + t_["lead"] < nqk)
        wo_ok = (nwo < npv * G and t >= pv_end[nwo // G] + t_["l_pw"]
                 and (nv >= H or nwo + t_["hold"] < nv))
        if s_ok:
            out.append(("s", ns))
            t += dur_a
            s_end[ns] = t
            ns += 1
        elif pv_ok:
            out.append(("pv", npv))
            t += dur_a
            pv_end[npv] = t
            npv += 1
        else:
            cand = [c for c, ok in (("qk", qk_ok), ("v", v_ok), ("wo", wo_ok)) if ok]
            if not cand:
                t += 4
                continue
            rot = {"qk": ("v", "wo", "qk"), "v": ("wo", "qk", "v"), "wo": ("qk", "v", "wo"),
                   None: ("qk", "v", "wo")}[last]
            last = [c for c in rot if c in cand][0]
            if last == "qk":
                out.append(("qk", nqk))
                t += dur_qk[nqk]
                qk_end[nqk] = t
                nqk += 1
            elif last == "v":
                out.append(("v", nv))
                t += dur_v[nv]
                v_end[nv] = t
                nv += 1
            else:
                out.append(("wo", nwo))
                t += dur_wo
                nwo += 1
    return out


NXC = 4
HI = 4
UP = 3
NA, NB = 2, 5
HA0, PA0 = 10, 7
HB0, PB0 = HA0 + HI * NA, PA0 + UP * NA


def _groups(npairs):
    g = [(0, 1), (1, 2), (3, 2), (5, 2)] + [(PA0 + UP * it, UP) for it in range(NA)]
    g += [(PB0 + 2 * UP * it, 2 * UP) for it in range(NB)]
    g += [(PB0 + 2 * UP * NB, npairs - PB0 - 2 * UP * NB)]
    return g


SEM_XS, SEM_X, SEM_O, SEM_O2, SEM_XB, SEM_WO, SEM_FFN, SEM_W = 0, 4, 5, 6, 7, 8, 9, 10


def _kernel(x_hbm, mem0_hbm, wq_hbm, wk_hbm, wv_hbm, wo_hbm, wr_hbm, wg_hbm, wu_hbm, wd_hbm,
            out_hbm,
            x_ref, xs_ref, xp_scr, raw_scr, w_ref, wo_ref, wg_ref, wu_ref, wd_ref,
            pre_scr, xn_scr, xa_scr, xc_scr, xb_scr, ot_scr, pin_scr, out_v, ks_scr, vs_scr,
            mem0_ref, wr_ref, zero_smem, sems,
            *, S, D, H, DH, M):
    L = M + SEG
    L0 = L - PR
    LM = L - VB
    KV = M + VB
    nseg = S // SEG
    nblk = nseg // U
    HP = H // 2
    NC = D // DH
    NPRE = 2 * H
    NFH = NFILL * (U - 1)
    fill_heads = list(range(H - NFH, H))
    xc = nseg // NXC
    groups = _groups(3 * HP)
    qscale = float(np.asarray(DH ** -0.5).astype(BF16)) * LOG2E
    neg = -1e9 * LOG2E

    def start_xs(c):
        pltpu.make_async_copy(x_hbm.at[c * xc:(c + 1) * xc, SEG - PR:SEG, :],
                              xs_ref.at[c * xc:(c + 1) * xc], sems.at[SEM_XS + min(c, 2)]).start()

    start_xs(0)
    start_xs(1)
    XA = U + 1
    early_cps = [pltpu.make_async_copy(x_hbm.at[0:XA], x_ref.at[0:XA], sems.at[SEM_X]),
                 pltpu.make_async_copy(mem0_hbm, mem0_ref, sems.at[SEM_X]),
                 pltpu.make_async_copy(wr_hbm, wr_ref, sems.at[SEM_X])]
    cp_xb = pltpu.make_async_copy(x_hbm.at[XA:nseg], x_ref.at[XA:nseg], sems.at[SEM_XB])
    w32 = [w.bitcast(U32) for w in (wq_hbm, wk_hbm, wv_hbm)]
    for gi, (g0, gn) in enumerate(groups):
        for i in range(g0, g0 + gn):
            pltpu.make_async_copy(w32[i // HP].at[:, i % HP, :], raw_scr.at[i], sems.at[SEM_W + gi]).start()
            if i == 0:
                start_xs(2)
                start_xs(3)
            if i == 30:
                for cp in early_cps:
                    cp.start()
    cp_wo = pltpu.make_async_copy(wo_hbm.bitcast(U32), wo_ref, sems.at[SEM_WO])
    cp_wo.start()
    cp_xb.start()
    ffn_cps = [pltpu.make_async_copy(src.bitcast(U32), dst, sems.at[SEM_FFN])
               for src, dst in ((wg_hbm, wg_ref), (wu_hbm, wu_ref), (wd_hbm, wd_ref))]
    for cp in ffn_cps:
        cp.start()
    zero_smem[0] = 0

    def wait_group(gi, g0, gn):
        blk = raw_scr.at[pl.ds(g0, gn)]
        pltpu.make_async_copy(blk, blk, sems.at[SEM_W + gi]).wait()

    def unpack(i):
        for cb in range(D // 128):
            a = raw_scr[i, pl.ds(cb * 128, 64, stride=2), :]
            b = raw_scr[i, pl.ds(cb * 128 + 1, 64, stride=2), :]
            w_ref[2 * i, cb * 64:(cb + 1) * 64, :] = (a & jnp.uint32(0xFFFF)) | (b << 16)
            w_ref[2 * i + 1, cb * 64:(cb + 1) * 64, :] = (a >> 16) | (b & jnp.uint32(0xFFFF0000))

    def tail_rows(segs):
        parts = [xn_scr[pl.ds(_mult(S + sg * SEG + (SEG - PR), PR), PR), :] for sg in segs]
        return jnp.concatenate(parts, axis=0)

    def sel_rows(seg0):
        return tail_rows([seg0 + u for u in range(U)]).astype(BF16)

    def fill(i, lhs, prow):
        pre_scr[NPRE + i, pl.ds(prow, U * PR), :] = _dot(lhs, _w(w_ref[2 * H + fill_heads[i]]))

    def wait_xs(c, n):
        blk = xs_ref.at[pl.ds(c * xc, n * xc)]
        pltpu.make_async_copy(blk, blk, sems.at[SEM_XS + c]).wait()

    def ln_sel(c):
        xv = xs_ref[pl.ds(c * xc, xc)].astype(F32).reshape(xc * PR, D)
        xp_scr[pl.ds(_mult(c * xc * PR, xc * PR), xc * PR), :] = _ln(xv).astype(BF16)

    def ln_body(c, carry):
        wait_xs(c, 1)
        ln_sel(c)
        return carry

    lax.fori_loop(0, 2, ln_body, 0)
    pin_scr[...] = jnp.zeros_like(pin_scr)
    for scr in (ks_scr, vs_scr):
        scr[0:8, :] = jnp.zeros((8, DH), F32)
    for u in range(U):
        r = S + u * SEG + (SEG - PR)
        xn_scr[r:r + PR, :] = jnp.zeros((PR, D), F32)
    wait_group(0, *groups[0])
    unpack(0)
    wait_xs(2, 2)
    half = 2 * xc * PR
    for e in range(2):
        pre_scr[e, 0:half, :] = _dot(xp_scr[0:half, :], _w(w_ref[e]))
    ln_sel(2)
    ln_sel(3)
    for e in range(2):
        pre_scr[e, half:2 * half, :] = _dot(xp_scr[half:2 * half, :], _w(w_ref[e]))

    def pre_iter(hd0, nh, gi, g0, gn, now=0):
        wait_group(gi, g0, gn)
        xp = xp_scr[...]
        pairs = [g0 + e for e in range(gn)]
        for i in pairs[:now]:
            unpack(i)
        pairs = pairs[now:]
        for e in range(nh):
            pre_scr[hd0 + e, 0:nseg * PR, :] = _dot(xp, _w(w_ref[hd0 + e]))
            if e >= 1:
                take = -(-len(pairs) // (nh - e))
                for i in pairs[:take]:
                    unpack(i)
                pairs = pairs[take:]

    def pre_a(it, carry):
        pre_iter(HA0 + HI * it, HI, 4 + it, PA0 + UP * it, UP)
        return carry

    def pre_b(it, carry):
        pre_iter(HB0 + 2 * HI * it, 2 * HI, 4 + NA + it, PB0 + 2 * UP * it, 2 * UP)
        return carry

    dz = zero_smem[0]
    pre_iter(2, 2, 1, groups[1][0] + dz, groups[1][1], now=1)
    pre_iter(4, 2, 2, groups[2][0] + dz, groups[2][1])
    pre_iter(6, HI, 3, groups[3][0] + dz, groups[3][1])
    lax.fori_loop(0, NA, pre_a, 0)
    lax.fori_loop(0, NB, pre_b, 0)
    for cp in early_cps:
        cp.wait()
    pre_iter(HB0 + 2 * HI * NB, NPRE - HB0 - 2 * HI * NB, len(groups) - 1, groups[-1][0] + dz, groups[-1][1])
    xn_scr[0:SEG, :] = _ln(x_ref[0].astype(F32))
    lhs0 = xp_scr[0:U * PR, :]
    for i in range(NFH):
        fill(i, lhs0, 0)
    cp_wo.wait()

    wr = wr_ref[...].astype(F32).reshape(1, D)
    rr = lax.broadcasted_iota(jnp.int32, (LM, L), 0)
    cc = lax.broadcasted_iota(jnp.int32, (LM, L), 1)
    mask = (rr < M) | (rr + VB >= cc)
    row8 = lax.broadcasted_iota(jnp.int32, (VB, DH), 0)
    shifts = list(range(0, M + 1)) + list(range(-1, -VB, -1))

    def vpu_attention(hd, qb, ch):
        b0 = 8 + KV * hd
        qs = qb * qscale
        ss = []
        for o in shifts:
            sv = jnp.sum(qs * ks_scr[b0 + o:b0 + o + VB, :], axis=-1, keepdims=True)
            sv = jnp.broadcast_to(sv, (VB, DH))
            if o < 0:
                sv = jnp.where(row8 >= -o, sv, neg)
            ss.append(sv)
        mx = den = acc = None
        for c0 in range(0, len(shifts), ch):
            cs = ss[c0:c0 + ch]
            cm = _tree(jnp.maximum, cs if mx is None else cs + [mx])
            if mx is not None:
                alpha = jnp.exp2(mx - cm)
                den = den * alpha
                acc = acc * alpha
            mx = cm
            for sv, o in zip(cs, shifts[c0:c0 + ch]):
                pv = jnp.exp2(sv - mx)
                t = pv * vs_scr[b0 + o:b0 + o + VB, :]
                den = pv if den is None else den + pv
                acc = t if acc is None else acc + t
        return acc * pl.reciprocal(den, approx=True)

    OB = U * SEG

    def out_copy(r0, nrows, sem):
        return pltpu.make_async_copy(out_v.at[pl.ds(r0, nrows)], out_hbm.at[pl.ds(r0, nrows)], sems.at[sem])

    def layer(li):
        first = li == 0
        base = li * S
        t_ = TUNE[li]
        order = _step_order(H, [2 * L0 if first else (L0 if hd < NP2 else L) + L for hd in range(H)],
                            [L0 if hd in fill_heads else L for hd in range(H)], LM, L, t_)
        plag, pgap = t_["plag"], t_["pgap"]
        pin_at = sorted(set(list(range(plag, H - pgap, t_["pstep"])) + [H - pgap - 1]))

        def finish(sp, o_tok, best_v, best_s, valid):
            r0 = _mult(sp * SEG, SEG)
            xin = x_ref[sp].astype(F32) if first else xb_scr[pl.ds(r0, SEG), :]
            x1 = _rb(xin + o_tok)
            xn1 = _ln(x1)
            r = _rb(jnp.sum(xn1 * wr, axis=-1, keepdims=True))
            upd = r > best_v
            if valid is not None:
                upd = jnp.logical_and(upd, valid)
            best_v = jnp.where(upd, r, best_v)
            best_s = jnp.where(upd, sp, best_s)
            x2 = _rb(x1 + xn1)
            xa_scr[pl.ds(r0, SEG), :] = x1
            if first:
                xc_scr[pl.ds(r0, SEG), :] = xn1
                xb_scr[pl.ds(r0, SEG), :] = x2
                xn_scr[pl.ds(S + r0, SEG), :] = _ln(x2)
            else:
                xn_scr[pl.ds(r0, SEG), :] = xn1
                out_v[pl.ds(r0, SEG), :] = x2.astype(BF16)
            return best_v, best_s

        def segment(s, mem, prev_tok, best_v, best_s, valid):
            r0 = pl.multiple_of(base + s * SEG, SEG)
            p0 = pl.multiple_of(s * PR, PR)
            h = jnp.concatenate([mem, xn_scr[pl.ds(r0, SEG), :]], axis=0)
            hb = h[:L0].astype(BF16)
            q, k, v, p, o, dd = ([None] * H for _ in range(6))
            acc = None
            nacc = 0
            za = pl.multiple_of((s >> 12) * 8, 8)
            zb = pl.multiple_of((s >> 13) * 8, 8)

            def proj(wi, slot):
                if slot is None:
                    return _dot(h, _w(w_ref[wi]))
                return jnp.concatenate([_dot(hb, _w(w_ref[wi])), pre_scr[slot, pl.ds(p0, PR), :]], axis=0)

            for kind, i in order:
                if kind == "qk":
                    q[i] = proj(i, i if (first or i < NP2) else None)
                    k[i] = proj(H + i, H + i if first else None)
                    ks_scr[8 + KV * i:8 + KV * (i + 1), :] = k[i][:KV]
                elif kind == "s":
                    for hd in range(i * G, (i + 1) * G):
                        qm = jnp.concatenate([q[hd][:M], q[hd][KV:]], axis=0)
                        sc = jnp.where(mask, _dot_nt(qm, k[hd]) * qscale, neg)
                        e = jnp.exp2(sc - jnp.max(sc, axis=-1, keepdims=True))
                        pn = e * pl.reciprocal(jnp.sum(e, axis=-1, keepdims=True), approx=True)
                        p[hd] = pn.astype(BF16)
                elif kind == "v":
                    v[i] = proj(2 * H + i, NPRE + fill_heads.index(i) if i in fill_heads else None)
                    vs_scr[8 + KV * i:8 + KV * (i + 1), :] = v[i][:KV]
                elif kind == "pv":
                    for hd in range(i * G, (i + 1) * G):
                        o[hd] = _dot(p[hd], v[hd])
                elif kind == "wo":
                    ov = vpu_attention(i, q[i][M:KV], t_["ch"])
                    top = o[i][:M]
                    if i - pgap in pin_at:
                        top = top + pin_scr[pl.ds(zb, 8), 0:DH]
                    lhs = jnp.concatenate([top, ov, o[i][M:]], axis=0)
                    dd[i] = jnp.concatenate(
                        [_dot(lhs, _w(wo_ref[i * (DH // 2):(i + 1) * (DH // 2), c * DH:(c + 1) * DH]))
                         for c in range(NC)], axis=1)
                    if i in pin_at:
                        while nacc <= i - plag:
                            acc = dd[nacc] if acc is None else acc + dd[nacc]
                            nacc += 1
                        pin_scr[pl.ds(za + 8, L), :] = acc
                else:
                    sp = s - 1 if valid is None else jnp.maximum(s - 1, 0)
                    best_v, best_s = finish(sp, prev_tok, best_v, best_s, valid)
                    if first:
                        sn = jnp.minimum(s + 1, nseg - 1)
                        xn_scr[pl.ds(pl.multiple_of(sn * SEG, SEG), SEG), :] = _ln(x_ref[sn].astype(F32))
                    h = jnp.concatenate([mem, xn_scr[pl.ds(r0, SEG), :]], axis=0)
                    hb = h[:L0].astype(BF16)
            for j in range(nacc, H):
                acc = acc + dd[j]
            res = _rb(acc)
            return res[:M], res[M:], best_v, best_s

        def block(b, carry):
            mem, best_v, best_s = carry
            if first:
                @pl.when(b == 1)
                def _():
                    cp_xb.wait()
            else:
                @pl.when(b >= 2)
                def _():
                    out_copy(pl.multiple_of((b - 2) * OB, OB), OB, SEM_O).start()
            tok = ot_scr[...]
            nb = jnp.minimum(b + 1, nblk - 1)
            for u in range(U):
                s = b * U + u
                mem, tok, best_v, best_s = segment(s, mem, tok, best_v, best_s, (s > 0) if u == 0 else None)
                if u < U - 1:
                    prow = (b + 1) * U * PR
                    if first:
                        lhs = xp_scr[pl.ds(pl.multiple_of(nb * U * PR, U * PR), U * PR), :]
                        lhs = jnp.where(b == nblk - 1, sel_rows(0), lhs)
                        prow = jnp.where(b == nblk - 1, 0, prow)
                    else:
                        lhs = sel_rows(nb * U)
                    for i in range(u * NFILL, (u + 1) * NFILL):
                        fill(i, lhs, pl.multiple_of(prow, U * PR))
            ot_scr[...] = tok
            return mem, best_v, best_s

        ot_scr[...] = jnp.zeros_like(ot_scr)
        init = (mem0_ref[...].astype(F32),
                jnp.full((SEG, 1), -jnp.inf, F32),
                jnp.zeros((SEG, 1), jnp.int32))
        _, best_v, best_s = lax.fori_loop(0, nblk, block, init)

        def ahead(hd):
            pre_scr[hd, 0:(nseg - 2) * PR, :] = _dot(tail_rows(range(nseg - 2)), _w(w_ref[hd]))

        if first:
            for cp in ffn_cps:
                cp.wait()
            ahead(0)
        best_v, best_s = finish(nseg - 1, ot_scr[...], best_v, best_s, None)
        if not first:
            out_copy((nblk - 2) * OB, 2 * OB, SEM_O).start()

        vmax = jnp.max(best_v, axis=0, keepdims=True)
        tok = best_s * SEG + lax.broadcasted_iota(jnp.int32, (SEG, 1), 0)
        idx = jnp.min(jnp.where(best_v == vmax, tok, S))
        idx = jnp.clip(idx, 0, S - 1)
        xs = xc_scr[pl.ds(idx, 1), :] if first else xn_scr[pl.ds(idx, 1), :]
        x1 = xa_scr[pl.ds(idx, 1), :]
        xs8 = jnp.broadcast_to(xs, (8, D))
        g = _rb(_dot(xs8, _w(wg_ref[...])))
        u = _rb(_dot(xs8, _w(wu_ref[...])))
        g = _rb(g * _rb(jax.nn.sigmoid(g)))
        y = _rb(_dot(_rb(g * u), _w(wd_ref[...])))
        if first:
            for hd in range(1, NP2):
                ahead(hd)
        y = _rb(y * _rb(jax.nn.sigmoid(vmax)))
        return idx, _rb(x1 + _rb(xs + y[0:1]))

    idx, new = layer(0)
    xb_scr[pl.ds(idx, 1), :] = new
    xn_scr[pl.ds(S + idx, 1), :] = _ln(new)
    sg = idx // SEG
    rows = tail_rows([nseg - 2, nseg - 1, sg])
    for hd in range(NP2):
        fx = _dot(rows, _w(w_ref[hd]))
        pre_scr[hd, (nseg - 2) * PR:nseg * PR, :] = fx[:2 * PR]
        pre_scr[hd, pl.ds(pl.multiple_of(sg * PR, PR), PR), :] = fx[2 * PR:]

    @pl.when(idx < U * SEG)
    def _():
        lhs = sel_rows(0)
        for i in range(NFH):
            fill(i, lhs, 0)

    idx, new = layer(1)
    out_copy(0, S, SEM_O).wait()
    b0 = pl.multiple_of((idx // 16) * 16, 16)
    blk = out_v[pl.ds(b0, 16), :].astype(F32)
    rid = b0 + lax.broadcasted_iota(jnp.int32, (16, D), 0)
    out_v[pl.ds(b0, 16), :] = jnp.where(rid == idx, new, blk).astype(BF16)
    cp = out_copy(b0, 16, SEM_O2)
    cp.start()
    cp.wait()


@jax.jit
def pallas_interleave_layers__memory_aug_recurrent_mem_tr__moe_arch_mod__prompt_kernel(
    A_x, A_mem0, A_Wq, A_Wk, A_Wv, A_Wo, A_seg_len, B_x, B_w_r, B_w_gate, B_w_up, B_w_down,
):
    B, S, D = A_x.shape
    _, H, DH = A_Wq.shape
    M = A_mem0.shape[1]
    F = B_w_gate.shape[1]
    assert (B, S, D, H, DH, M) == (1, 2048, 512, 32, 128, 8)
    nseg = S // SEG
    kern = functools.partial(_kernel, S=S, D=D, H=H, DH=DH, M=M)
    hbm = pl.BlockSpec(memory_space=pl.ANY)
    out = pl.pallas_call(
        kern,
        out_shape=jax.ShapeDtypeStruct((S, D), BF16),
        in_specs=[hbm] * 10,
        out_specs=hbm,
        scratch_shapes=[
            pltpu.VMEM((nseg, SEG, D), BF16),
            pltpu.VMEM((nseg, PR, D), BF16),
            pltpu.VMEM((nseg * PR, D), BF16),
            pltpu.VMEM((3 * (H // 2), D, DH), U32),
            pltpu.VMEM((3 * H, D // 2, DH), U32),
            pltpu.VMEM((H * DH // 2, D), U32),
            pltpu.VMEM((D // 2, F), U32), pltpu.VMEM((D // 2, F), U32), pltpu.VMEM((F // 2, D), U32),
            pltpu.VMEM((2 * H + NFILL * (U - 1), (nseg + U) * PR, DH), F32),
            pltpu.VMEM((2 * S, D), F32),
            pltpu.VMEM((S, D), F32), pltpu.VMEM((S, D), F32), pltpu.VMEM((S, D), F32),
            pltpu.VMEM((SEG, D), F32),
            pltpu.VMEM((M + SEG + 8, D), F32),
            pltpu.VMEM((S, D), BF16),
            pltpu.VMEM((8 + H * (M + VB), DH), F32), pltpu.VMEM((8 + H * (M + VB), DH), F32),
            pltpu.VMEM((M, D), BF16), pltpu.VMEM((D,), BF16),
            pltpu.SMEM((1,), jnp.int32),
            pltpu.SemaphoreType.DMA((SEM_W + len(_groups(3 * (H // 2))),))],
        compiler_params=pltpu.CompilerParams(vmem_limit_bytes=110 * 1024 * 1024),
    )(A_x.reshape(nseg, SEG, D), A_mem0.reshape(M, D), A_Wq, A_Wk, A_Wv,
      A_Wo.reshape(H * DH, D), B_w_r, B_w_gate, B_w_up, B_w_down)
    return out.reshape(B, S, D)
```
